```python
import os as _os
_os.environ.setdefault("JAX_PLATFORMS", "cpu")
import jax
import jax.numpy as jnp

def _softmax(x, axis=-1):
    return jax.nn.softmax(x, axis=axis)
def _gelu(x):
    return jax.nn.gelu(x, approximate=True)
def _silu(x):
    return jax.nn.silu(x)
def _sigmoid(x):
    return jax.nn.sigmoid(x)
def _layernorm(x, axis=-1, eps=1e-5):
    m = jnp.mean(x, axis=axis, keepdims=True)
    v = jnp.var(x, axis=axis, keepdims=True)
    return (x - m) / jnp.sqrt(v + eps)
def _scatter_add(tgt, idx, src, axis=0):
    return tgt.at[idx].add(src)
def _segment_sum(src, seg, n):
    return jax.ops.segment_sum(src, seg, n)
class _Rng:
    def __init__(self, key):
        self._k = key
    def _next(self):
        self._k, sub = jax.random.split(self._k)
        return sub
    def normal(self, shape):
        return jax.random.normal(self._next(), shape, dtype=jnp.bfloat16)
    def randint(self, lo, hi, shape):
        return jax.random.randint(self._next(), shape, lo, hi, dtype=jnp.int32)
    def uniform(self, shape, lo=0.0, hi=1.0):
        return jax.random.uniform(self._next(), shape, jnp.bfloat16, lo, hi)
    def permutation(self, n):
        return jax.random.permutation(self._next(), n)


kernel_name = 'sequential_preLN__sliding_block__dense_activation_relu__prompt'

def setup_inputs():
    _rng = _Rng(jax.random.key(int.from_bytes(__import__("os").urandom(4), "little")))
    _w = (lambda a: (lambda t: t.astype(jnp.bfloat16) if jnp.issubdtype(t.dtype, jnp.floating) else t)(jnp.asarray(a)))
    def _A_setup():
        B, S, D = 1, 2048, 640
        return {
            "x": _w((lambda *s: _rng.normal(s) * 0.05)(B, S, D)),
            "wqkv": _w((lambda *s: _rng.normal(s) * 0.05)(D, 3 * D)),
            "wo": _w((lambda *s: _rng.normal(s) * 0.05)(D, D)),
        }
    _A_in = _A_setup()

    def _B_setup():
        B, S, D, Dff = 1, 2048, 640, 1536
        return {
            "x": _w((lambda *s: _rng.normal(s) * 0.05)(B, S, D)),
            "w1": _w((lambda *s: _rng.normal(s) * 0.05)(D, Dff)),
            "w2": _w((lambda *s: _rng.normal(s) * 0.05)(Dff, D)),
        }
    _B_in = _B_setup()

    return {
        "A_x": _A_in["x"],
        "A_wqkv": _A_in["wqkv"],
        "A_wo": _A_in["wo"],
        "B_x": _B_in["x"],
        "B_w1": _B_in["w1"],
        "B_w2": _B_in["w2"],
    }

def reference(A_x, A_wqkv, A_wo, B_x, B_w1, B_w2):
    def _A_ref(x, wqkv, wo):
        B, S, D = x.shape
        H = 32; Dh = D // H; W = 256
        qkv = (lambda x, *d: x.transpose(*d))((x @ wqkv).reshape(B, S, 3, H, Dh), 2, 0, 3, 1, 4)
        q, k, v = qkv[0], qkv[1], qkv[2]
        scores = jnp.einsum("bhqd,bhkd->bhqk", q, k) * (Dh ** -0.5)
        idx = jnp.arange(S)
        mask = (idx[:, None] - idx[None, :] >= 0) & (idx[:, None] - idx[None, :] < W)
        scores = jnp.where(mask[None, None], scores, -1e9)
        p = _softmax(scores, axis=-1)
        o = jnp.einsum("bhqk,bhkd->bhqd", p, v)
        return (lambda x, *d: x.transpose(*d))(o, 0, 2, 1, 3).reshape(B, S, D) @ wo

    def _B_ref(x, w1, w2):
        h = jnp.einsum("bsd,df->bsf", x, w1)
        zero = jnp.zeros_like(h)
        h = jnp.maximum(h, zero)
        return jnp.einsum("bsf,fd->bsd", h, w2)

    x = A_x
    h = x + _A_ref(_layernorm(x, axis=-1), A_wqkv, A_wo)
    h2 = h + _B_ref(_layernorm(h, axis=-1), B_w1, B_w2)
    return h2
```

```python
import functools
import math

import jax
import jax.numpy as jnp
import jax.experimental.pallas as pl
import jax.experimental.pallas.tpu as pltpu

S = 2048
D = 640
H = 32
DH = 20
W = 256
DFF = 1536
NG = 8
T = 256
NB = T // 128
NSTEP = S // T
VR = H * 8
DEPTH = 2
EPS = 1e-5
NEG = -1e9 * math.log2(math.e)
NT = (((1,), (1,)), ((), ()))
F32 = jnp.float32
BF16 = jnp.bfloat16
U32 = jnp.uint32
QKC = 256
NQK = 2 * D // QKC


def _ln(x):
    m = jnp.mean(x, axis=-1, keepdims=True)
    xc = x - m
    v = jnp.mean(xc * xc, axis=-1, keepdims=True)
    return xc * jax.lax.rsqrt(v + EPS)


def _pack(x):
    return pltpu.bitcast(x.astype(BF16), U32)


def _unpack(x):
    return pltpu.bitcast(x, BF16)


def _pack2(a, b):
    return pltpu.pack_elementwise([a, b], packed_dtype=BF16)


def _group_tile(a, g, lane):
    o = (80 * g) % 128
    t0 = (80 * g) // 128
    lo = a[:, t0 * 128:(t0 + 1) * 128]
    if o + 80 <= 128:
        return lo
    return jnp.where(lane >= o, lo, a[:, (t0 + 1) * 128:(t0 + 2) * 128])


def _dot(a, b):
    return jnp.dot(a, b, preferred_element_type=F32)


def _kernel(x_ref, wqkv_hbm, wo_hbm, w1_hbm, w2_hbm, o_ref,
            wqkv_ref, wo_ref, w1_ref, w2_ref, sems,
            wvt_ref, k_ref, vt_ref, q_ref, hres_ref, hn_ref):
    i = pl.program_id(0)

    def copies():
        cs = [pltpu.make_async_copy(wqkv_hbm.at[:, c * QKC:(c + 1) * QKC],
                                    wqkv_ref.at[:, c * QKC:(c + 1) * QKC], sems.at[c])
              for c in range(NQK)]
        cs.append(pltpu.make_async_copy(wqkv_hbm.at[:, 2 * D:3 * D],
                                        wqkv_ref.at[:, 2 * D:3 * D], sems.at[NQK]))
        cs.append(pltpu.make_async_copy(wo_hbm, wo_ref, sems.at[NQK + 1]))
        cs.append(pltpu.make_async_copy(w1_hbm, w1_ref, sems.at[NQK + 2]))
        cs.append(pltpu.make_async_copy(w2_hbm, w2_ref, sems.at[NQK + 3]))
        return cs

    def ffn_up():
        hn = _unpack(hn_ref[...])
        return jnp.maximum(_dot(hn, w1_ref[...]), 0.0).astype(BF16)

    def ffn_down(h1, c0, c1):
        cols = slice(c0 * 128, c1 * 128)
        out = hres_ref[:, cols] + _dot(h1, w2_ref[:, cols])
        o_ref[0, :, cols] = out.astype(o_ref.dtype)

    def body(first):
        lane1 = jax.lax.broadcasted_iota(jnp.int32, (1, 128), 1)
        r32 = jax.lax.broadcasted_iota(jnp.int32, (32, 128), 0)
        l32 = jax.lax.broadcasted_iota(jnp.int32, (32, 128), 1)
        tri = r32 <= (l32 & 31)
        odd = (lane1 & 32) != 0
        hi = (lane1 & 64) != 0
        row8 = jax.lax.broadcasted_iota(jnp.int32, (8, 128), 0)
        zero = jnp.zeros((16, 128), U32)
        ones8 = jnp.ones((8, 128), F32)
        if first:
            cs = copies()
            for c in cs:
                c.start()
            row0, vrow0 = 0, 0
        else:
            row0 = pl.multiple_of(i * (T // 2), T // 2)
            vrow0 = pl.multiple_of(i * (NB * VR), VR)
            h1 = ffn_up()

        x = x_ref[0].astype(F32)
        xnf = _ln(x)
        xn = xnf.astype(BF16)
        xni = _unpack(jnp.concatenate(
            [_pack2(xnf[32 * m:32 * m + 16], xnf[32 * m + 16:32 * m + 32])
             for m in range(T // 32)], axis=0))
        if first:
            parts = []
            for c in range(NQK):
                cs[c].wait()
                parts.append(_dot(xn, wqkv_ref[:, c * QKC:(c + 1) * QKC]))
            qk = jnp.concatenate(parts, axis=1)
            cs[NQK].wait()
            wvt_ref[...] = _pack(wqkv_ref[:, 2 * D:3 * D].astype(F32).T)
        else:
            qk = _dot(xn, wqkv_ref[:, 0:2 * D])
        vt = jax.lax.dot_general(_unpack(wvt_ref[...]), xni, NT, preferred_element_type=F32)

        q = qk[:, 0:D] * (DH ** -0.5 * math.log2(math.e))
        k = qk[:, D:2 * D]
        for g in range(NG):
            k_ref[pl.ds(row0, T // 2), g * 128:(g + 1) * 128] = _pack(_group_tile(k, g, lane1))
            q_ref[:, g * 128:(g + 1) * 128] = _pack(_group_tile(q, g, lane1))
        for tb in range(NB):
            for hh in range(2):
                parts = []
                for h in range(hh * 16, hh * 16 + 16):
                    w0 = (DH * h) // 16 * 16
                    if h % 4 < 2:
                        parts += [vt[w0:w0 + 24, tb * 128:(tb + 1) * 128], ones8]
                    else:
                        parts += [ones8, vt[w0 + 8:w0 + 32, tb * 128:(tb + 1) * 128]]
                vt_ref[pl.ds(vrow0 + tb * VR, VR), hh * 128:(hh + 1) * 128] = _pack(
                    jnp.concatenate(parts, axis=0))

        def skip(b, j):
            return max(0, 8 - 4 * b - j) if first else 0

        def scores(b, g):
            off = (80 * g) % 128
            f = (lane1 - off) & 127
            hm = [(f >= 20 * h) & (f < 20 * h + 20) for h in range(4)]
            ss, es, ms = [], [], []
            for j in range(4):
                r0 = skip(b, j)
                qj = q_ref[b * 64 + j * 16:b * 64 + j * 16 + 16, g * 128:(g + 1) * 128]
                qbd = jnp.concatenate(
                    [jnp.where(hm[(c - j) % 4], qj, zero) for c in range(4)], axis=0)
                kw = k_ref[pl.ds(row0 + (b * 64 + j * 16 - 128 + r0 * 16), (9 - r0) * 16),
                           g * 128:(g + 1) * 128]
                s = jax.lax.dot_general(_unpack(kw), _unpack(qbd), NT,
                                        preferred_element_type=F32)
                blocks = [None] * r0 + [s[32 * r:32 * r + 32] for r in range(9 - r0)]
                edge = jnp.where(tri, blocks[8], NEG if r0 else blocks[0])
                t = [edge] + [blocks[r] for r in range(max(r0, 1), 8)]
                while len(t) > 1:
                    t = ([jnp.maximum(t[a], t[a + 1]) for a in range(0, len(t) - 1, 2)]
                         + t[len(t) & ~1:])
                t = jnp.maximum(jnp.maximum(t[0][0:8], t[0][8:16]),
                                jnp.maximum(t[0][16:24], t[0][24:32]))
                ms.append(jnp.max(t, axis=0, keepdims=True))
                es.append(edge)
                ss.append(blocks)
            return ss, es, ms

        def sel(mk, a, bb):
            if a is None and bb is None:
                return None
            return jnp.where(mk, zero if a is None else a, zero if bb is None else bb)

        def pv(b, g, sem):
            ss, es, ms = sem
            pes = [None] * 4
            accs = [None] * 4
            for kt in range(3):
                if first and b + kt < 2:
                    continue
                heads = [[] for _ in range(4)]
                for blk in range(4 * kt, 4 * kt + 4):
                    src = []
                    for j in range(4):
                        r = blk - j
                        if not skip(b, j) <= r < 9:
                            src.append(None)
                            continue
                        if r in (0, 8) and pes[j] is None:
                            pes[j] = jnp.exp2(es[j] - ms[j])
                        if r == 0:
                            p = jnp.where(tri, 0.0, pes[j])
                        elif r == 8:
                            p = jnp.where(tri, pes[j], 0.0) if not skip(b, j) else pes[j]
                        else:
                            p = jnp.exp2(ss[j][r] - ms[j])
                        src.append(_pack2(p[0:16], p[16:32]))
                    t = [sel(odd, src[(j + 1) % 4], src[j]) for j in range(4)]
                    for h in range(4):
                        j = (-h) % 4
                        v = sel(hi, t[(j + 2) % 4], t[j])
                        heads[h].append(zero if v is None else v)
                for h in range(4):
                    pw = _unpack(jnp.concatenate(heads[h], axis=0))
                    vv = _unpack(vt_ref[
                        pl.ds(vrow0 + ((b + kt - 2) * VR + (4 * (g % 4) + h) * 16), 16),
                        (g // 4) * 128:(g // 4 + 1) * 128])
                    d = _dot(vv, pw)
                    accs[h] = d if accs[h] is None else accs[h] + d
            os_ = []
            for h in range(4):
                acc = accs[h]
                if h < 2:
                    den, num = acc[24:32], acc[0:24]
                else:
                    den, num = acc[0:8], acc[8:32]
                inv = pl.reciprocal(den, approx=True)
                inv = inv * (2.0 - den * inv)
                num = num * jnp.concatenate([inv, inv, inv], axis=0)
                if h:
                    num = pltpu.roll(num, (128 - 32 * h) % 128, 1)
                os_.append(num)
            o0, o1, o2, o3 = os_
            return [o0[0:16], jnp.where(row8 < 4, o0[16:24], o1[0:8]), o1[8:24],
                    o2[0:16], jnp.where(row8 < 4, o2[16:24], o3[0:8]), o3[8:24]]

        if not first:
            ffn_down(h1, 0, 1)
        items = [(b, g) for b in range(NB) for g in range(NG)]
        ot_parts = [[] for _ in range(NB)]
        o_blocks = []
        sq = [scores(*items[n]) for n in range(DEPTH)]
        for n, (b, g) in enumerate(items):
            if n + DEPTH < len(items):
                sq.append(scores(*items[n + DEPTH]))
            elif not first:
                c = 1 + n + DEPTH - len(items)
                ffn_down(h1, c, c + 1)
            ot_parts[b] += pv(b, g, sq[n])
            if g == NG - 1:
                ot = jnp.concatenate(ot_parts[b], axis=0)
                o_blocks.append(ot.T.astype(BF16))
        o = jnp.concatenate(o_blocks, axis=0)
        if first:
            cs[NQK + 1].wait()
        else:
            ffn_down(h1, 3, 4)
        hres = x + _dot(o, wo_ref[...])
        if not first:
            ffn_down(h1, 4, 5)
        hres_ref[...] = hres
        hn_ref[...] = _pack(_ln(hres))
        if first:
            cs[NQK + 2].wait()
            cs[NQK + 3].wait()

    @pl.when(i == 0)
    def _():
        body(True)

    @pl.when(jnp.logical_and(i > 0, i < NSTEP))
    def _():
        body(False)

    @pl.when(i == NSTEP)
    def _():
        ffn_down(ffn_up(), 0, 5)


@jax.jit
def pallas_sequential_preLN__sliding_block__dense_activation_relu__prompt_kernel(A_x, A_wqkv, A_wo, B_x, B_w1, B_w2):
    del B_x
    hbm = pl.BlockSpec(memory_space=pl.ANY)
    return pl.pallas_call(
        _kernel,
        grid=(NSTEP + 1,),
        in_specs=[
            pl.BlockSpec((1, T, D), lambda i: (0, jnp.minimum(i, NSTEP - 1), 0)),
            hbm, hbm, hbm, hbm,
        ],
        out_specs=pl.BlockSpec((1, T, D), lambda i: (0, jnp.maximum(i - 1, 0), 0)),
        out_shape=jax.ShapeDtypeStruct((1, S, D), BF16),
        scratch_shapes=[
            pltpu.VMEM((D, 3 * D), BF16),
            pltpu.VMEM((D, D), BF16),
            pltpu.VMEM((D, DFF), BF16),
            pltpu.VMEM((DFF, D), BF16),
            pltpu.SemaphoreType.DMA((NQK + 4,)),
            pltpu.VMEM((D // 2, D), U32),
            pltpu.VMEM((S // 2, NG * 128), U32),
            pltpu.VMEM((S // 128 * VR, 256), U32),
            pltpu.VMEM((T // 2, NG * 128), U32),
            pltpu.VMEM((T, D), F32),
            pltpu.VMEM((T // 2, D), U32),
        ],
        compiler_params=pltpu.CompilerParams(
            dimension_semantics=("arbitrary",),
            vmem_limit_bytes=100 * 1024 * 1024),
        name="fused_block",
    )(A_x, A_wqkv, A_wo, B_w1, B_w2)
```

```python
import functools
import math

import jax
import jax.numpy as jnp
import jax.experimental.pallas as pl
import jax.experimental.pallas.tpu as pltpu

S = 2048
D = 640
H = 32
DH = 20
DFF = 1536
NG = 8
T = 256
NB = T // 128
NI = NB * NG
NSTEP = S // T
VR = H * 24
DEPTH = 7
LOOK = 2
EPS = 1e-5
NEG = -1e9 * math.log2(math.e)
QSCALE = DH ** -0.5 * math.log2(math.e)
NT = (((1,), (1,)), ((), ()))
F32 = jnp.float32
BF16 = jnp.bfloat16
U32 = jnp.uint32
GTILE = (0, 5, 1, 6, 7, 3, 8, 4)
MERGE = {1: (5, 80), 2: (6, 112), 3: (7, 64), 4: (8, 96)}
WCH = ((5, 7), (7, 10), (10, 15), (0, 5))
NW = len(WCH)
OCH = ((0, 128), (128, 224), (224, 256))
PROW = 256
MROW = 448


def _ln(x):
    m = jnp.mean(x, axis=-1, keepdims=True)
    xc = x - m
    v = jnp.mean(xc * xc, axis=-1, keepdims=True)
    return xc * jax.lax.rsqrt(v + EPS)


def _pack(x):
    return pltpu.bitcast(x.astype(BF16), U32)


def _unpack(x):
    return pltpu.bitcast(x, BF16)


def _pack2(a, b):
    return pltpu.pack_elementwise([a, b], packed_dtype=BF16)


def _pack_keys(x):
    return jnp.concatenate([_pack2(x[r:r + 16], x[r + 16:r + 32])
                            for r in range(0, x.shape[0], 32)], axis=0)


def _colmax(t):
    mx = t[0]
    for a in t[1:]:
        mx = jnp.maximum(mx, a)
    mx = jnp.maximum(jnp.maximum(mx[0:8], mx[8:16]), jnp.maximum(mx[16:24], mx[24:32]))
    return jnp.max(mx, axis=0, keepdims=True)


def _dot5(a, w_ref, c0, c1):
    m = a.shape[0]
    outs = []
    c4 = c0 + (c1 - c0) // 4 * 4
    if c4 > c0:
        outs.append(jnp.dot(a, w_ref[:, c0 * 128:c4 * 128], preferred_element_type=F32))
    for c in range(c4, c1):
        w = w_ref[512:640, c * 128:(c + 1) * 128]
        last = jnp.concatenate(
            [jnp.dot(a[r:r + m // 4, 512:640], w, preferred_element_type=F32)
             for r in range(0, m, m // 4)], axis=0)
        outs.append(jnp.dot(a[:, 0:512], w_ref[0:512, c * 128:(c + 1) * 128],
                            preferred_element_type=F32) + last)
    return outs[0] if len(outs) == 1 else jnp.concatenate(outs, axis=1)


def _tile(t, n=1):
    return slice(t * 128, (t + n) * 128)


def _mo(v, m):
    return v if isinstance(v, int) else pl.multiple_of(v, m)


def _kernel(x_hbm, wqkv_hbm, wo_hbm, w1_hbm, w2_hbm, o_hbm,
            o_ref, x_ref, wqkv_ref, wo_ref, w1_ref, w2_ref, isems, osems,
            wvt_ref, xn_ref, xni_ref, k_ref, vt_ref, q_ref, hres_ref, hn_ref, h1_ref,
            z_ref, *sp_refs):
    step = pl.program_id(0)

    def wcopies():
        cs = [pltpu.make_async_copy(wqkv_hbm.at[:, a * 128:b * 128],
                                    wqkv_ref.at[:, a * 128:b * 128], isems.at[n])
              for n, (a, b) in enumerate(WCH)]
        cs.append(pltpu.make_async_copy(wo_hbm, wo_ref, isems.at[NW]))
        cs.append(pltpu.make_async_copy(w1_hbm, w1_ref, isems.at[NW + 1]))
        cs.append(pltpu.make_async_copy(w2_hbm, w2_ref, isems.at[NW + 2]))
        return cs

    def xcopy(blk):
        slot = blk % 2
        return pltpu.make_async_copy(x_hbm.at[0, pl.ds(_mo(blk * T, T), T), :],
                                     x_ref.at[pl.ds(_mo(slot * T, T), T), :],
                                     isems.at[NW + 3 + slot])

    def ocopy(row, n, sem):
        return pltpu.make_async_copy(o_ref.at[pl.ds(row, n), :],
                                     o_hbm.at[0, pl.ds(row, n), :], osems.at[sem])

    def stage(st):
        static = isinstance(st, int)
        first = static and st == 0
        lane1 = jax.lax.broadcasted_iota(jnp.int32, (1, 128), 1)
        row8 = jax.lax.broadcasted_iota(jnp.int32, (8, 128), 0)

        def store_vt(blk, vt, c, tb):
            parts = []
            for w0 in range(0, 160, 40):
                mid = vt[w0 + 16:w0 + 24]
                parts += [vt[w0:w0 + 16], jnp.where(row8 < 4, mid, 1.0),
                          jnp.where(row8 < 4, 1.0, mid), vt[w0 + 24:w0 + 40]]
            vt_ref[pl.ds(_mo((blk * NB + tb) * VR + c * 192, 8), 192), :] = (
                jnp.concatenate(parts, axis=0))

        def v_proj(blk, xni):
            for half in range(2):
                vt = jax.lax.dot_general(_unpack(wvt_ref[160 * half:160 * half + 160, :]), xni,
                                         NT, preferred_element_type=F32)
                for c in range(2):
                    for tb in range(NB):
                        store_vt(blk, vt[160 * c:160 * c + 160, _tile(tb)], 2 * half + c, tb)

        def ffn_up(c0, c1):
            a = _dot5(_unpack(hn_ref[...]), w1_ref, c0, c1)
            h1_ref[:, _tile(c0, c1 - c0)] = _pack(jnp.maximum(a, 0.0))

        def ffn_down(c0, c1, r0, r1):
            cols = _tile(c0, c1 - c0)
            a = jnp.dot(_unpack(h1_ref[r0 // 2:r1 // 2, :]), w2_ref[:, cols],
                        preferred_element_type=F32)
            out = hres_ref[pl.ds(_mo(((st + 1) % 2) * T + r0, 32), r1 - r0), cols] + a
            o_ref[pl.ds(_mo((st - 1) * T + r0, 32), r1 - r0), cols] = out.astype(BF16)

        if static and st == NSTEP:
            ffn_up(0, DFF // 128)
            base = (st - 1) * T
            for n, (r0, r1) in enumerate(OCH):
                ffn_down(0, 5, r0, r1)
                ocopy(base + r0, r1 - r0, NSTEP - 1 + n).start()
            for blk in range(NSTEP - 1):
                ocopy(blk * T, T, blk).wait()
            for n, (r0, r1) in enumerate(OCH):
                ocopy(base + r0, r1 - r0, NSTEP - 1 + n).wait()
            return

        def out_proj(b, ot):
            rows = pl.ds(_mo((st % 2) * T + b * 128, 128), 128)
            hres = x_ref[rows, :].astype(F32) + _dot5(ot, wo_ref, 0, 5)
            hres_ref[rows, :] = hres
            hn_ref[b * 64:(b + 1) * 64, :] = _pack(_ln(hres))

        z_ref[0] = 0
        zoff = pl.multiple_of(z_ref[0], 8)
        r32 = jax.lax.broadcasted_iota(jnp.int32, (32, 128), 0)
        l32 = jax.lax.broadcasted_iota(jnp.int32, (32, 128), 1)
        tri = r32 <= (l32 & 31)
        r16 = jax.lax.broadcasted_iota(jnp.int32, (16, 128), 0)
        l16 = jax.lax.broadcasted_iota(jnp.int32, (16, 128), 1) & 31
        trim = (jnp.where(r16 <= l16, jnp.uint32(0xFFFF), jnp.uint32(0))
                | jnp.where(r16 + 16 <= l16, jnp.uint32(0xFFFF0000), jnp.uint32(0)))
        odd = (lane1 & 32) != 0
        hi = (lane1 & 64) != 0
        zero = jnp.zeros((16, 128), U32)
        qrow0 = T // 2 if static and st == 1 else 0

        def skip(n, j):
            return max(0, 8 - 4 * (n // NG) - j) if first else 0

        def scores(n):
            b, g = n // NG, n % NG
            sp = sp_refs[n]
            f = (lane1 - (80 * g) % 128) & 127
            hm = [(f >= 20 * h) & (f < 20 * h + 20) for h in range(4)]
            cols = _tile(GTILE[g])
            for j in range(4):
                r0 = skip(n, j)
                q0 = qrow0 + b * 64 + j * 16
                qj = q_ref[q0:q0 + 16, cols]
                qbd = jnp.concatenate(
                    [jnp.where(hm[(c - j) % 4], qj, zero) for c in range(4)], axis=0)
                diag = st * (T // 2) + b * 64 + j * 16
                kw = k_ref[pl.ds(_mo(diag, 16), 16), cols]
                if r0 < 8:
                    kw = jnp.concatenate(
                        [kw, k_ref[pl.ds(_mo(diag - (8 - r0) * 16, 16), (8 - r0) * 16), cols]],
                        axis=0)
                s = jax.lax.dot_general(_unpack(kw), _unpack(qbd), NT,
                                        preferred_element_type=F32)
                if r0:
                    t = [jnp.where(tri, s[0:32], NEG)] + [
                        s[32 * r:32 * r + 32] for r in range(1, 9 - r0)]
                else:
                    t = [jnp.where(tri, s[0:32], s[32:64])] + [
                        s[32 * r:32 * r + 32] for r in range(2, 9)]
                sp[0:32 * len(t), _tile(j)] = pltpu.bitcast(jnp.concatenate(t, axis=0), U32)
                sp[MROW:MROW + 8, _tile(j)] = pltpu.bitcast(
                    jnp.broadcast_to(_colmax(t), (8, 128)), U32)

        def sel(mk, a, b):
            if a is None and b is None:
                return None
            return jnp.where(mk, zero if a is None else a, zero if b is None else b)

        def probs(n):
            sp = sp_refs[n]
            mx = [pltpu.bitcast(sp[MROW:MROW + 8, _tile(j)], F32)[0:1] for j in range(4)]

            def load(blk):
                out = []
                for j in range(4):
                    r, r0 = blk - j, skip(n, j)
                    if not r0 <= r < 9 or (r == 8 and not r0):
                        out.append(None)
                        continue
                    rr = 0 if r in (0, 8) else r - max(r0 - 1, 0)
                    out.append(pltpu.bitcast(sp[pl.ds(zoff + 32 * rr, 32), _tile(j)], F32))
                return out

            blks = [blk for blk in range(12) if not (first and n // NG + blk // 4 < 2)]
            loaded = {blk: load(blk) for blk in blks[:LOOK]}
            edge = [None] * 4
            for idx, blk in enumerate(blks):
                src = []
                for j in range(4):
                    s = loaded[blk][j]
                    if s is not None:
                        p = jnp.exp2(s - mx[j])
                        p = _pack2(p[0:16], p[16:32])
                        if blk == j:
                            edge[j] = p
                            p = p & ~trim
                        src.append(p)
                    elif blk - j == 8:
                        src.append(edge[j] & trim)
                    else:
                        src.append(None)
                t = [sel(odd, src[(j + 1) % 4], src[j]) for j in range(4)]
                for h in range(4):
                    v = sel(hi, t[(2 - h) % 4], t[(-h) % 4])
                    sp[PROW + 16 * blk:PROW + 16 * blk + 16, _tile(h)] = zero if v is None else v
                if idx + LOOK < len(blks):
                    loaded[blks[idx + LOOK]] = load(blks[idx + LOOK])

        def pv(n):
            b, g = n // NG, n % NG
            sp = sp_refs[n]
            accs = [None] * 4
            for kt in range(3):
                if first and b + kt < 2:
                    continue
                for h in range(4):
                    pw = _unpack(sp[PROW + 64 * kt:PROW + 64 * kt + 64, _tile(h)])
                    vrow = (st * NB + b + kt - 2) * VR + (4 * g + h) * 24
                    d = jnp.dot(vt_ref[pl.ds(_mo(vrow, 8), 24), :], pw,
                                preferred_element_type=F32)
                    accs[h] = d if accs[h] is None else accs[h] + d
            out = []
            for h in (0, 2):
                ev, od = accs[h], accs[h + 1]
                den = jnp.where(row8 < 4, od[0:8], ev[16:24])
                inv = pl.reciprocal(den, approx=True)
                inv = inv * (2.0 - den * inv)
                rot = pltpu.roll(inv, 4, 0)
                iev = jnp.where(row8 < 4, rot, inv)
                iod = jnp.where(row8 < 4, inv, rot)
                ev = ev * jnp.concatenate([iev, iev, iev], axis=0)
                od = od * jnp.concatenate([iod, iod, iod], axis=0)
                if h:
                    ev = pltpu.roll(ev, 128 - 32 * h, 1)
                od = pltpu.roll(od, 128 - 32 * (h + 1), 1)
                out += [ev[0:16], jnp.where(row8 < 4, ev[16:24], od[0:8]), od[8:24]]
            return out

        ot_parts = [[] for _ in range(NB)]

        def attn_out(b):
            return jnp.concatenate(ot_parts[b], axis=0).T.astype(BF16)

        if first:
            def ln1(blk):
                xnf = _ln(x_ref[blk * T:(blk + 1) * T, :].astype(F32))
                rows = slice(blk * (T // 2), (blk + 1) * (T // 2))
                xn_ref[rows, :] = _pack(xnf)
                xni_ref[rows, :] = _pack_keys(xnf)

            def qk_proj(which, b0, b1, t0, t1):
                rows = slice(b0 * (T // 2), b1 * (T // 2))
                col0 = (0 if which == "q" else 5) + t0
                a = _dot5(_unpack(xn_ref[rows, :]), wqkv_ref, col0, col0 + t1 - t0)
                ref = q_ref if which == "q" else k_ref
                if which == "q":
                    a = a * QSCALE
                ref[rows, _tile(t0, t1 - t0)] = _pack(a)
                for t in range(max(t0, 1), t1):
                    dst, split = MERGE[t]
                    ref[rows, _tile(dst)] = jnp.where(lane1 >= split, ref[rows, _tile(t - 1)],
                                                      ref[rows, _tile(t)])

            cs = wcopies()
            xcopy(0).start()
            xcopy(1).start()
            for c in cs:
                c.start()
            xcopy(0).wait()
            ln1(0)
            xcopy(1).wait()
            ln1(1)
            cs[0].wait()
            qk_proj("k", 0, 2, 0, 2)
            cs[1].wait()
            qk_proj("k", 0, 2, 2, 5)
            cs[2].wait()
            v = [_dot5(_unpack(xni_ref[64 * tb:64 * tb + 64, :]), wqkv_ref, 10, 15)
                 for tb in range(NB)]
            wvt_ref[...] = _pack(wqkv_ref[:, 2 * D:3 * D].astype(F32).T)
            v_proj(1, _unpack(xni_ref[T // 2:T, :]))
            for tb in range(NB):
                vt = v[tb].T
                for c in range(4):
                    store_vt(0, vt[160 * c:160 * c + 160], c, tb)
            cs[3].wait()
            cs[4].wait()
            qk_proj("q", 0, 1, 0, 5)
            for n in range(NI):
                scores(n)
            for n in range(NI):
                probs(n)
                ot_parts[n // NG] += pv(n)
                if n in (0, 9, 13):
                    t = (0, 9, 13).index(n)
                    qk_proj("q", 1, 2, t, t + 1)
                if n == NG + 3:
                    out_proj(0, attn_out(0))
            qk_proj("q", 1, 2, 3, 4)
            out_proj(1, attn_out(1))
            qk_proj("q", 1, 2, 4, 5)
            cs[5].wait()
            cs[6].wait()
            return

        def next_x(fn):
            if static:
                fn()
            else:
                pl.when(st + 1 < NSTEP)(fn)

        next_x(lambda: xcopy(st + 1).start())
        if static:
            up0 = 1
            ffn_up(0, up0)
        else:
            up0 = 3
            ffn_up(0, up0)
            xnf = _ln(x_ref[pl.ds(_mo((st % 2) * T, T), T), :].astype(F32))
            qk = _dot5(xnf.astype(BF16), wqkv_ref, 0, 10)
            q = qk[:, 0:D] * QSCALE
            k = qk[:, D:2 * D]
            v_proj(st, _unpack(_pack_keys(xnf)))
            krows = pl.ds(_mo(st * (T // 2), T // 2), T // 2)
            for g in range(NG):
                t0, off = (80 * g) // 128, (80 * g) % 128
                for a, ref, rows in ((k, k_ref, krows), (q, q_ref, pl.ds(0, T // 2))):
                    v = a[:, _tile(t0)]
                    if off + 80 > 128:
                        v = jnp.where(lane1 >= off, v, a[:, _tile(t0 + 1)])
                    ref[rows, _tile(GTILE[g])] = _pack(v)
        queue = [functools.partial(ffn_up, c, c + 1) for c in range(up0, DFF // 128)]
        nup = len(queue)
        queue += [functools.partial(ffn_down, c, c + 1, r, r + 128)
                  for c in range(3) for r in (0, 128)]
        done = 0

        def fill(upto):
            nonlocal done
            while done < min(upto, len(queue)):
                queue[done]()
                done += 1

        for n in range(DEPTH):
            scores(n)
        o_blocks = []
        for n in range(NI):
            if n + DEPTH < NI:
                scores(n + DEPTH)
            probs(n)
            ot_parts[n // NG] += pv(n)
            fill(-(-(n + 1) * len(queue) // NI))
            if n % NG == NG - 1:
                o_blocks.append(attn_out(n // NG))
            if n == NG + 1:
                fill(nup)
                out_proj(0, o_blocks[0])
        ffn_down(3, 4, 0, T)
        out_proj(1, o_blocks[1])
        ffn_down(4, 5, 0, 128)
        ffn_down(4, 5, 128, T)
        ocopy(_mo((st - 1) * T, T), T, st - 1).start()
        next_x(lambda: xcopy(st + 1).wait())

    pl.when(step == 0)(lambda: stage(0))
    pl.when(step == 1)(lambda: stage(1))
    pl.when(jnp.logical_and(step > 1, step < NSTEP))(lambda: stage(step))
    pl.when(step == NSTEP)(lambda: stage(NSTEP))


@jax.jit
def pallas_sequential_preLN__sliding_block__dense_activation_relu__prompt_kernel(A_x, A_wqkv, A_wo, B_x, B_w1, B_w2):
    del B_x
    hbm = pl.BlockSpec(memory_space=pl.ANY)
    return pl.pallas_call(
        _kernel,
        grid=(NSTEP + 1,),
        in_specs=[hbm, hbm, hbm, hbm, hbm],
        out_specs=hbm,
        out_shape=jax.ShapeDtypeStruct((1, S, D), BF16),
        scratch_shapes=[
            pltpu.VMEM((S, D), BF16),
            pltpu.VMEM((2 * T, D), BF16),
            pltpu.VMEM((D, 3 * D), BF16),
            pltpu.VMEM((D, D), BF16),
            pltpu.VMEM((D, DFF), BF16),
            pltpu.VMEM((DFF, D), BF16),
            pltpu.SemaphoreType.DMA((NW + 5,)),
            pltpu.SemaphoreType.DMA((NSTEP - 1 + len(OCH),)),
            pltpu.VMEM((D // 2, D), U32),
            pltpu.VMEM((T, D), U32),
            pltpu.VMEM((T, D), U32),
            pltpu.VMEM((S // 2, 9 * 128), U32),
            pltpu.VMEM((S // 128 * VR, 128), F32),
            pltpu.VMEM((T, 9 * 128), U32),
            pltpu.VMEM((2 * T, D), F32),
            pltpu.VMEM((T // 2, D), U32),
            pltpu.VMEM((T // 2, DFF), U32),
            pltpu.SMEM((1,), jnp.int32),
        ] + [pltpu.VMEM((MROW + 8, 512), U32)] * NI,
        compiler_params=pltpu.CompilerParams(
            dimension_semantics=("arbitrary",),
            vmem_limit_bytes=100 * 1024 * 1024),
        name="fused_block",
    )(A_x, A_wqkv, A_wo, B_w1, B_w2)
```

```python
import functools
import math

import jax
import jax.numpy as jnp
import jax.experimental.pallas as pl
import jax.experimental.pallas.tpu as pltpu

S = 2048
D = 640
H = 32
DH = 20
DFF = 1536
NG = 8
T = 256
NB = T // 128
NI = NB * NG
NSTEP = S // T
VR = H * 24
DEPTH = 7
LOOK = 2
RS = 16
EPS = 1e-5
NEG = -1e9 * math.log2(math.e)
QSCALE = DH ** -0.5 * math.log2(math.e)
NT = (((1,), (1,)), ((), ()))
F32 = jnp.float32
BF16 = jnp.bfloat16
U32 = jnp.uint32
GTILE = (0, 5, 1, 6, 7, 3, 8, 4)
MERGE = {1: (5, 80), 2: (6, 112), 3: (7, 64), 4: (8, 96)}
WCH = ((5, 7), (7, 10), (10, 15), (0, 5))
NW = len(WCH)
OCH = ((0, 128), (128, 224), (224, 256))
PROW = 256
MROW = 448


def _ln(x):
    m = jnp.mean(x, axis=-1, keepdims=True)
    xc = x - m
    v = jnp.mean(xc * xc, axis=-1, keepdims=True)
    return xc * jax.lax.rsqrt(v + EPS)


def _pack(x):
    return pltpu.bitcast(x.astype(BF16), U32)


def _unpack(x):
    return pltpu.bitcast(x, BF16)


def _colmax(t):
    mx = t[0]
    for a in t[1:]:
        mx = jnp.maximum(mx, a)
    mx = jnp.maximum(jnp.maximum(mx[0:8], mx[8:16]), jnp.maximum(mx[16:24], mx[24:32]))
    return jnp.max(mx, axis=0, keepdims=True)


def _dot5(a, w_ref, c0, c1):
    m = a.shape[0]
    outs = []
    c4 = c0 + (c1 - c0) // 4 * 4
    if c4 > c0:
        outs.append(jnp.dot(a, w_ref[:, c0 * 128:c4 * 128], preferred_element_type=F32))
    for c in range(c4, c1):
        w = w_ref[512:640, c * 128:(c + 1) * 128]
        last = jnp.concatenate(
            [jnp.dot(a[r:r + m // 4, 512:640], w, preferred_element_type=F32)
             for r in range(0, m, m // 4)], axis=0)
        outs.append(jnp.dot(a[:, 0:512], w_ref[0:512, c * 128:(c + 1) * 128],
                            preferred_element_type=F32) + last)
    return outs[0] if len(outs) == 1 else jnp.concatenate(outs, axis=1)


def _tile(t, n=1):
    return slice(t * 128, (t + n) * 128)


def _mo(v, m):
    return v if isinstance(v, int) else pl.multiple_of(v, m)


def _kernel(x_hbm, wqkv_hbm, wo_hbm, w1_hbm, w2_hbm, o_hbm,
            o_ref, x_ref, wqkv_ref, wo_ref, w1_ref, w2_ref, isems, osems,
            wvt_ref, xn_ref, k_ref, vt_ref, q_ref, hres_ref, hn_ref, h1_ref,
            z_ref, *sp_refs):
    step = pl.program_id(0)

    def wcopies():
        cs = [pltpu.make_async_copy(wqkv_hbm.at[:, a * 128:b * 128],
                                    wqkv_ref.at[:, a * 128:b * 128], isems.at[n])
              for n, (a, b) in enumerate(WCH)]
        cs.append(pltpu.make_async_copy(wo_hbm, wo_ref, isems.at[NW]))
        cs.append(pltpu.make_async_copy(w1_hbm, w1_ref, isems.at[NW + 1]))
        cs.append(pltpu.make_async_copy(w2_hbm, w2_ref, isems.at[NW + 2]))
        return cs

    def xcopy(blk):
        slot = blk % 2
        return pltpu.make_async_copy(x_hbm.at[0, pl.ds(_mo(blk * T, T), T), :],
                                     x_ref.at[pl.ds(_mo(slot * T, T), T), :],
                                     isems.at[NW + 3 + slot])

    def ocopy(row, n, sem):
        return pltpu.make_async_copy(o_ref.at[pl.ds(row, n), :],
                                     o_hbm.at[0, pl.ds(row, n), :], osems.at[sem])

    def stage(st):
        static = isinstance(st, int)
        first = static and st == 0
        lane1 = jax.lax.broadcasted_iota(jnp.int32, (1, 128), 1)
        row8 = jax.lax.broadcasted_iota(jnp.int32, (8, 128), 0)

        def store_vt(blk, vt, c, tb):
            parts = []
            for w0 in range(0, 160, 40):
                mid = vt[w0 + 16:w0 + 24]
                parts += [vt[w0:w0 + 16], jnp.where(row8 < 4, mid, 1.0),
                          jnp.where(row8 < 4, 1.0, mid), vt[w0 + 24:w0 + 40]]
            vt_ref[pl.ds(_mo((blk * NB + tb) * VR + c * 192, 8), 192), :] = (
                jnp.concatenate(parts, axis=0))

        def v_proj(blk, xn):
            for half in range(2):
                vt = jax.lax.dot_general(_unpack(wvt_ref[160 * half:160 * half + 160, :]), xn,
                                         NT, preferred_element_type=F32)
                for c in range(2):
                    for tb in range(NB):
                        store_vt(blk, vt[160 * c:160 * c + 160, _tile(tb)], 2 * half + c, tb)

        def ffn_up(c0, c1):
            a = _dot5(_unpack(hn_ref[...]), w1_ref, c0, c1)
            h1_ref[:, _tile(c0, c1 - c0)] = _pack(jnp.maximum(a, 0.0))

        def ffn_down(c0, c1, r0, r1):
            cols = _tile(c0, c1 - c0)
            a = jnp.dot(_unpack(h1_ref[r0 // 2:r1 // 2, :]), w2_ref[:, cols],
                        preferred_element_type=F32)
            out = hres_ref[pl.ds(_mo(((st + 1) % 2) * T + r0, 32), r1 - r0), cols] + a
            o_ref[pl.ds(_mo((st - 1) * T + r0, 32), r1 - r0), cols] = out.astype(BF16)

        if static and st == NSTEP:
            ffn_up(0, DFF // 128)
            base = (st - 1) * T
            for n, (r0, r1) in enumerate(OCH):
                ffn_down(0, 5, r0, r1)
                ocopy(base + r0, r1 - r0, NSTEP - 1 + n).start()
            for blk in range(NSTEP - 1):
                ocopy(blk * T, T, blk).wait()
            for n, (r0, r1) in enumerate(OCH):
                ocopy(base + r0, r1 - r0, NSTEP - 1 + n).wait()
            return

        def out_proj(b, ot):
            rows = pl.ds(_mo((st % 2) * T + b * 128, 128), 128)
            hres = x_ref[rows, :].astype(F32) + _dot5(ot, wo_ref, 0, 5)
            hres_ref[rows, :] = hres
            hn_ref[b * 64:(b + 1) * 64, :] = _pack(_ln(hres))

        z_ref[0] = 0
        zoff = pl.multiple_of(z_ref[0], 8)
        r32 = jax.lax.broadcasted_iota(jnp.int32, (32, 128), 0)
        l32 = jax.lax.broadcasted_iota(jnp.int32, (32, 128), 1)
        tri = r32 <= (l32 & 31)
        odd = (lane1 & 32) != 0
        hi = (lane1 & 64) != 0
        zero = jnp.zeros((16, 128), U32)
        qrow0 = T // 2 if static and st == 1 else 0

        def skip(n, j):
            return max(0, 8 - 4 * (n // NG) - j) if first else 0

        def scores(n):
            b, g = n // NG, n % NG
            sp = sp_refs[n]
            f = (lane1 - (80 * g) % 128) & 127
            hm = [(f >= 20 * h) & (f < 20 * h + 20) for h in range(4)]
            cols = _tile(GTILE[g])
            for j in range(4):
                r0 = skip(n, j)
                q0 = qrow0 + b * 64 + j * 16
                qj = q_ref[q0:q0 + 16, cols]
                qbd = jnp.concatenate(
                    [jnp.where(hm[(c - j) % 4], qj, zero) for c in range(4)], axis=0)
                diag = st * (T // 2) + b * 64 + j * 16
                kw = k_ref[pl.ds(_mo(diag, 16), 16), cols]
                if r0 < 8:
                    kw = jnp.concatenate(
                        [kw, k_ref[pl.ds(_mo(diag - (8 - r0) * 16, 16), (8 - r0) * 16), cols]],
                        axis=0)
                s = jax.lax.dot_general(_unpack(kw), _unpack(qbd), NT,
                                        preferred_element_type=F32)
                if r0:
                    t = [jnp.where(tri, s[0:32], NEG)] + [
                        s[32 * r:32 * r + 32] for r in range(1, 9 - r0)]
                else:
                    t = [jnp.where(tri, s[0:32], s[32:64])] + [
                        s[32 * r:32 * r + 32] for r in range(2, 9)]
                sp[0:32 * len(t), _tile(j)] = pltpu.bitcast(jnp.concatenate(t, axis=0), U32)
                sp[MROW:MROW + 8, _tile(j)] = pltpu.bitcast(
                    jnp.broadcast_to(_colmax(t), (8, 128)), U32)

        def sel(mk, a, b):
            if a is None and b is None:
                return None
            return jnp.where(mk, 0.0 if a is None else a, 0.0 if b is None else b)

        def probs(n):
            sp = sp_refs[n]
            mx = [pltpu.bitcast(sp[MROW:MROW + 8, _tile(j)], F32)[0:1] for j in range(4)]

            def load(blk, half):
                out = []
                for j in range(4):
                    r, r0 = blk - j, skip(n, j)
                    if not r0 <= r < 9 or (r == 8 and not r0):
                        out.append(None)
                        continue
                    rr = 0 if r in (0, 8) else r - max(r0 - 1, 0)
                    out.append(pltpu.bitcast(
                        sp[pl.ds(zoff + (32 * rr + RS * half), RS), _tile(j)], F32))
                return out

            steps = [(blk, half) for blk in range(12) for half in range(32 // RS)
                     if not (first and n // NG + blk // 4 < 2)]
            loaded = {s: load(*s) for s in steps[:LOOK]}
            edge = {}
            for idx, (blk, half) in enumerate(steps):
                src = []
                for j in range(4):
                    s = loaded[blk, half][j]
                    if s is not None:
                        p = jnp.exp2(s - mx[j])
                        if blk == j:
                            m = tri[RS * half:RS * half + RS]
                            edge[j, half] = jnp.where(m, p, 0.0)
                            p = jnp.where(m, 0.0, p)
                        src.append(p)
                    else:
                        src.append(edge[j, half] if blk - j == 8 else None)
                t = [sel(odd, src[(j + 1) % 4], src[j]) for j in range(4)]
                row = PROW + 16 * blk + RS // 2 * half
                for h in range(4):
                    v = sel(hi, t[(2 - h) % 4], t[(-h) % 4])
                    sp[row:row + RS // 2, _tile(h)] = zero[0:RS // 2] if v is None else _pack(v)
                if idx + LOOK < len(steps):
                    loaded[steps[idx + LOOK]] = load(*steps[idx + LOOK])

        def pv(n):
            b, g = n // NG, n % NG
            sp = sp_refs[n]
            accs = [None] * 4
            for kt in range(3):
                if first and b + kt < 2:
                    continue
                for h in range(4):
                    pw = _unpack(sp[PROW + 64 * kt:PROW + 64 * kt + 64, _tile(h)])
                    vrow = (st * NB + b + kt - 2) * VR + (4 * g + h) * 24
                    d = jnp.dot(vt_ref[pl.ds(_mo(vrow, 8), 24), :], pw,
                                preferred_element_type=F32)
                    accs[h] = d if accs[h] is None else accs[h] + d
            out = []
            for h in (0, 2):
                ev, od = accs[h], accs[h + 1]
                den = jnp.where(row8 < 4, od[0:8], ev[16:24])
                inv = pl.reciprocal(den, approx=True)
                inv = inv * (2.0 - den * inv)
                rot = pltpu.roll(inv, 4, 0)
                iev = jnp.where(row8 < 4, rot, inv)
                iod = jnp.where(row8 < 4, inv, rot)
                ev = ev * jnp.concatenate([iev, iev, iev], axis=0)
                od = od * jnp.concatenate([iod, iod, iod], axis=0)
                if h:
                    ev = pltpu.roll(ev, 128 - 32 * h, 1)
                od = pltpu.roll(od, 128 - 32 * (h + 1), 1)
                out += [ev[0:16], jnp.where(row8 < 4, ev[16:24], od[0:8]), od[8:24]]
            return out

        ot_parts = [[] for _ in range(NB)]

        def attn_out(b):
            return jnp.concatenate(ot_parts[b], axis=0).T.astype(BF16)

        if first:
            def ln1(blk):
                xn_ref[blk * (T // 2):(blk + 1) * (T // 2), :] = _pack(
                    _ln(x_ref[blk * T:(blk + 1) * T, :].astype(F32)))

            def qk_proj(which, b0, b1, t0, t1):
                rows = slice(b0 * (T // 2), b1 * (T // 2))
                col0 = (0 if which == "q" else 5) + t0
                a = _dot5(_unpack(xn_ref[rows, :]), wqkv_ref, col0, col0 + t1 - t0)
                ref = q_ref if which == "q" else k_ref
                if which == "q":
                    a = a * QSCALE
                ref[rows, _tile(t0, t1 - t0)] = _pack(a)
                for t in range(max(t0, 1), t1):
                    dst, split = MERGE[t]
                    ref[rows, _tile(dst)] = jnp.where(lane1 >= split, ref[rows, _tile(t - 1)],
                                                      ref[rows, _tile(t)])

            cs = wcopies()
            xcopy(0).start()
            xcopy(1).start()
            for c in cs:
                c.start()
            xcopy(0).wait()
            ln1(0)
            xcopy(1).wait()
            ln1(1)
            cs[0].wait()
            qk_proj("k", 0, 2, 0, 2)
            cs[1].wait()
            qk_proj("k", 0, 2, 2, 5)
            cs[2].wait()
            v = [_dot5(_unpack(xn_ref[64 * tb:64 * tb + 64, :]), wqkv_ref, 10, 15)
                 for tb in range(NB)]
            wvt_ref[...] = _pack(wqkv_ref[:, 2 * D:3 * D].astype(F32).T)
            v_proj(1, _unpack(xn_ref[T // 2:T, :]))
            for tb in range(NB):
                vt = v[tb].T
                for c in range(4):
                    store_vt(0, vt[160 * c:160 * c + 160], c, tb)
            cs[3].wait()
            cs[4].wait()
            qk_proj("q", 0, 1, 0, 5)
            for n in range(NI):
                scores(n)
            for n in range(NI):
                probs(n)
                ot_parts[n // NG] += pv(n)
                if n in (0, 9, 13):
                    t = (0, 9, 13).index(n)
                    qk_proj("q", 1, 2, t, t + 1)
                if n == NG + 3:
                    out_proj(0, attn_out(0))
            qk_proj("q", 1, 2, 3, 4)
            out_proj(1, attn_out(1))
            qk_proj("q", 1, 2, 4, 5)
            cs[5].wait()
            cs[6].wait()
            return

        def next_x(fn):
            if static:
                fn()
            else:
                pl.when(st + 1 < NSTEP)(fn)

        next_x(lambda: xcopy(st + 1).start())
        if static:
            up0 = 1
            ffn_up(0, up0)
        else:
            up0 = 3
            ffn_up(0, up0)
            xn = _ln(x_ref[pl.ds(_mo((st % 2) * T, T), T), :].astype(F32)).astype(BF16)
            qk = _dot5(xn, wqkv_ref, 0, 10)
            q = qk[:, 0:D] * QSCALE
            k = qk[:, D:2 * D]
            v_proj(st, xn)
            krows = pl.ds(_mo(st * (T // 2), T // 2), T // 2)
            for g in range(NG):
                t0, off = (80 * g) // 128, (80 * g) % 128
                for a, ref, rows in ((k, k_ref, krows), (q, q_ref, pl.ds(0, T // 2))):
                    v = a[:, _tile(t0)]
                    if off + 80 > 128:
                        v = jnp.where(lane1 >= off, v, a[:, _tile(t0 + 1)])
                    ref[rows, _tile(GTILE[g])] = _pack(v)
        queue = [functools.partial(ffn_up, c, c + 1) for c in range(up0, DFF // 128)]
        nup = len(queue)
        queue += [functools.partial(ffn_down, c, c + 1, r, r + 128)
                  for c in range(3) for r in (0, 128)]
        done = 0

        def fill(upto):
            nonlocal done
            while done < min(upto, len(queue)):
                queue[done]()
                done += 1

        for n in range(DEPTH):
            scores(n)
        o_blocks = []
        for n in range(NI):
            if n + DEPTH < NI:
                scores(n + DEPTH)
            probs(n)
            ot_parts[n // NG] += pv(n)
            fill(-(-(n + 1) * len(queue) // NI))
            if n % NG == NG - 1:
                o_blocks.append(attn_out(n // NG))
            if n == NG + 1:
                fill(nup)
                out_proj(0, o_blocks[0])
        ffn_down(3, 4, 0, T)
        out_proj(1, o_blocks[1])
        ffn_down(4, 5, 0, 128)
        ffn_down(4, 5, 128, T)
        ocopy(_mo((st - 1) * T, T), T, st - 1).start()
        next_x(lambda: xcopy(st + 1).wait())

    pl.when(step == 0)(lambda: stage(0))
    pl.when(step == 1)(lambda: stage(1))
    pl.when(jnp.logical_and(step > 1, step < NSTEP))(lambda: stage(step))
    pl.when(step == NSTEP)(lambda: stage(NSTEP))


@jax.jit
def pallas_sequential_preLN__sliding_block__dense_activation_relu__prompt_kernel(A_x, A_wqkv, A_wo, B_x, B_w1, B_w2):
    del B_x
    hbm = pl.BlockSpec(memory_space=pl.ANY)
    return pl.pallas_call(
        _kernel,
        grid=(NSTEP + 1,),
        in_specs=[hbm, hbm, hbm, hbm, hbm],
        out_specs=hbm,
        out_shape=jax.ShapeDtypeStruct((1, S, D), BF16),
        scratch_shapes=[
            pltpu.VMEM((S, D), BF16),
            pltpu.VMEM((2 * T, D), BF16),
            pltpu.VMEM((D, 3 * D), BF16),
            pltpu.VMEM((D, D), BF16),
            pltpu.VMEM((D, DFF), BF16),
            pltpu.VMEM((DFF, D), BF16),
            pltpu.SemaphoreType.DMA((NW + 5,)),
            pltpu.SemaphoreType.DMA((NSTEP - 1 + len(OCH),)),
            pltpu.VMEM((D // 2, D), U32),
            pltpu.VMEM((T, D), U32),
            pltpu.VMEM((S // 2, 9 * 128), U32),
            pltpu.VMEM((S // 128 * VR, 128), F32),
            pltpu.VMEM((T, 9 * 128), U32),
            pltpu.VMEM((2 * T, D), F32),
            pltpu.VMEM((T // 2, D), U32),
            pltpu.VMEM((T // 2, DFF), U32),
            pltpu.SMEM((1,), jnp.int32),
        ] + [pltpu.VMEM((MROW + 8, 512), U32)] * NI,
        compiler_params=pltpu.CompilerParams(
            dimension_semantics=("arbitrary",),
            vmem_limit_bytes=100 * 1024 * 1024),
        name="fused_block",
    )(A_x, A_wqkv, A_wo, B_w1, B_w2)
```

```python
import functools
import math

import jax
import jax.numpy as jnp
import jax.experimental.pallas as pl
import jax.experimental.pallas.tpu as pltpu

S = 2048
D = 640
H = 32
DH = 20
DFF = 1536
NG = 8
T = 256
NB = T // 128
NI = NB * NG
NSTEP = S // T
VR = H * 24
DEPTH = 7
LOOK = 2
RS = 16
EPS = 1e-5
NEG = -1e9 * math.log2(math.e)
QSCALE = DH ** -0.5 * math.log2(math.e)
NT = (((1,), (1,)), ((), ()))
F32 = jnp.float32
BF16 = jnp.bfloat16
U32 = jnp.uint32
GTILE = (0, 5, 1, 6, 7, 3, 8, 4)
MERGE = {1: (5, 80), 2: (6, 112), 3: (7, 64), 4: (8, 96)}
WCH = ((5, 7), (7, 10), (10, 15), (0, 5))
NW = len(WCH)
OCH = ((0, 128), (128, 224), (224, 256))
PROW = 256
MROW = 448


def _ln(x):
    m = jnp.mean(x, axis=-1, keepdims=True)
    xc = x - m
    v = jnp.mean(xc * xc, axis=-1, keepdims=True)
    return xc * jax.lax.rsqrt(v + EPS)


def _pack(x):
    return pltpu.bitcast(x.astype(BF16), U32)


def _unpack(x):
    return pltpu.bitcast(x, BF16)


def _colmax(t):
    mx = t[0]
    for a in t[1:]:
        mx = jnp.maximum(mx, a)
    mx = jnp.maximum(jnp.maximum(mx[0:8], mx[8:16]), jnp.maximum(mx[16:24], mx[24:32]))
    return jnp.max(mx, axis=0, keepdims=True)


def _dot5(a, w_ref, c0, c1):
    m = a.shape[0]
    outs = []
    c4 = c0 + (c1 - c0) // 4 * 4
    if c4 > c0:
        outs.append(jnp.dot(a, w_ref[:, c0 * 128:c4 * 128], preferred_element_type=F32))
    for c in range(c4, c1):
        w = w_ref[512:640, c * 128:(c + 1) * 128]
        last = jnp.concatenate(
            [jnp.dot(a[r:r + m // 4, 512:640], w, preferred_element_type=F32)
             for r in range(0, m, m // 4)], axis=0)
        outs.append(jnp.dot(a[:, 0:512], w_ref[0:512, c * 128:(c + 1) * 128],
                            preferred_element_type=F32) + last)
    return outs[0] if len(outs) == 1 else jnp.concatenate(outs, axis=1)


def _tile(t, n=1):
    return slice(t * 128, (t + n) * 128)


def _mo(v, m):
    return v if isinstance(v, int) else pl.multiple_of(v, m)


def _kernel(x_hbm, wqkv_hbm, wo_hbm, w1_hbm, w2_hbm, o_hbm,
            o_ref, x_ref, wqkv_ref, wo_ref, w1_ref, w2_ref, isems, osems,
            wvt_ref, xn_ref, k_ref, vt_ref, q_ref, hres_ref, hn_ref, h1_ref,
            z_ref, *sp_refs):
    step = pl.program_id(0)

    def wcopies():
        cs = [pltpu.make_async_copy(wqkv_hbm.at[:, a * 128:b * 128],
                                    wqkv_ref.at[:, a * 128:b * 128], isems.at[n])
              for n, (a, b) in enumerate(WCH)]
        cs.append(pltpu.make_async_copy(wo_hbm, wo_ref, isems.at[NW]))
        cs.append(pltpu.make_async_copy(w1_hbm, w1_ref, isems.at[NW + 1]))
        cs.append(pltpu.make_async_copy(w2_hbm, w2_ref, isems.at[NW + 2]))
        return cs

    def xcopy(blk):
        slot = blk % 2
        return pltpu.make_async_copy(x_hbm.at[0, pl.ds(_mo(blk * T, T), T), :],
                                     x_ref.at[pl.ds(_mo(slot * T, T), T), :],
                                     isems.at[NW + 3 + slot])

    def ocopy(row, n, sem):
        return pltpu.make_async_copy(o_ref.at[pl.ds(row, n), :],
                                     o_hbm.at[0, pl.ds(row, n), :], osems.at[sem])

    def stage(st):
        static = isinstance(st, int)
        first = static and st == 0
        lane1 = jax.lax.broadcasted_iota(jnp.int32, (1, 128), 1)
        row8 = jax.lax.broadcasted_iota(jnp.int32, (8, 128), 0)

        def store_vt(blk, vt, c, tb):
            parts = []
            for w0 in range(0, 160, 40):
                mid = vt[w0 + 16:w0 + 24]
                parts += [vt[w0:w0 + 16], jnp.where(row8 < 4, mid, 1.0),
                          jnp.where(row8 < 4, 1.0, mid), vt[w0 + 24:w0 + 40]]
            vt_ref[pl.ds(_mo((blk * NB + tb) * VR + c * 192, 8), 192), :] = (
                jnp.concatenate(parts, axis=0))

        def v_proj(blk, xn):
            for half in range(2):
                vt = jax.lax.dot_general(_unpack(wvt_ref[160 * half:160 * half + 160, :]), xn,
                                         NT, preferred_element_type=F32)
                for c in range(2):
                    for tb in range(NB):
                        store_vt(blk, vt[160 * c:160 * c + 160, _tile(tb)], 2 * half + c, tb)

        def ffn_up(c0, c1):
            a = _dot5(_unpack(hn_ref[...]), w1_ref, c0, c1)
            h1_ref[:, _tile(c0, c1 - c0)] = _pack(jnp.maximum(a, 0.0))

        def ffn_down(c0, c1, r0, r1):
            cols = _tile(c0, c1 - c0)
            a = jnp.dot(_unpack(h1_ref[r0 // 2:r1 // 2, :]), w2_ref[:, cols],
                        preferred_element_type=F32)
            out = hres_ref[pl.ds(_mo(((st + 1) % 2) * T + r0, 32), r1 - r0), cols] + a
            o_ref[pl.ds(_mo((st - 1) * T + r0, 32), r1 - r0), cols] = out.astype(BF16)

        if static and st == NSTEP:
            ffn_up(0, DFF // 128)
            base = (st - 1) * T
            for n, (r0, r1) in enumerate(OCH):
                ffn_down(0, 5, r0, r1)
                ocopy(base + r0, r1 - r0, NSTEP - 1 + n).start()
            for blk in range(NSTEP - 1):
                ocopy(blk * T, T, blk).wait()
            for n, (r0, r1) in enumerate(OCH):
                ocopy(base + r0, r1 - r0, NSTEP - 1 + n).wait()
            return

        def out_proj(b, ot):
            rows = pl.ds(_mo((st % 2) * T + b * 128, 128), 128)
            hres = x_ref[rows, :].astype(F32) + _dot5(ot, wo_ref, 0, 5)
            hres_ref[rows, :] = hres
            hn_ref[b * 64:(b + 1) * 64, :] = _pack(_ln(hres))

        z_ref[0] = 0
        zoff = pl.multiple_of(z_ref[0], 8)
        r32 = jax.lax.broadcasted_iota(jnp.int32, (32, 128), 0)
        l32 = jax.lax.broadcasted_iota(jnp.int32, (32, 128), 1)
        tri = r32 <= (l32 & 31)
        odd = (lane1 & 32) != 0
        hi = (lane1 & 64) != 0
        zero = jnp.zeros((16, 128), U32)
        qrow0 = T // 2 if static and st == 1 else 0

        def skip(n, j):
            return max(0, 8 - 4 * (n // NG) - j) if first else 0

        def scores(n):
            b, g = n // NG, n % NG
            sp = sp_refs[n]
            f = (lane1 - (80 * g) % 128) & 127
            hm = [(f >= 20 * h) & (f < 20 * h + 20) for h in range(4)]
            cols = _tile(GTILE[g])
            for j in range(4):
                r0 = skip(n, j)
                q0 = qrow0 + b * 64 + j * 16
                qj = q_ref[q0:q0 + 16, cols]
                qbd = jnp.concatenate(
                    [jnp.where(hm[(c - j) % 4], qj, zero) for c in range(4)], axis=0)
                diag = st * (T // 2) + b * 64 + j * 16
                kw = k_ref[pl.ds(_mo(diag, 16), 16), cols]
                if r0 < 8:
                    kw = jnp.concatenate(
                        [kw, k_ref[pl.ds(_mo(diag - (8 - r0) * 16, 16), (8 - r0) * 16), cols]],
                        axis=0)
                s = jax.lax.dot_general(_unpack(kw), _unpack(qbd), NT,
                                        preferred_element_type=F32)
                if r0:
                    t = [jnp.where(tri, s[0:32], NEG)] + [
                        s[32 * r:32 * r + 32] for r in range(1, 9 - r0)]
                else:
                    t = [jnp.where(tri, s[0:32], s[32:64])] + [
                        s[32 * r:32 * r + 32] for r in range(2, 9)]
                sp[0:32 * len(t), _tile(j)] = pltpu.bitcast(jnp.concatenate(t, axis=0), U32)
                sp[MROW:MROW + 8, _tile(j)] = pltpu.bitcast(
                    jnp.broadcast_to(_colmax(t), (8, 128)), U32)

        def sel(mk, a, b):
            if a is None and b is None:
                return None
            return jnp.where(mk, 0.0 if a is None else a, 0.0 if b is None else b)

        def probs(n):
            sp = sp_refs[n]
            mx = [pltpu.bitcast(sp[MROW:MROW + 8, _tile(j)], F32)[0:1] for j in range(4)]

            def load(blk, half):
                out = []
                for j in range(4):
                    r, r0 = blk - j, skip(n, j)
                    if not r0 <= r < 9 or (r == 8 and not r0):
                        out.append(None)
                        continue
                    rr = 0 if r in (0, 8) else r - max(r0 - 1, 0)
                    out.append(pltpu.bitcast(
                        sp[pl.ds(zoff + (32 * rr + RS * half), RS), _tile(j)], F32))
                return out

            steps = [(blk, half) for blk in range(12) for half in range(32 // RS)
                     if not (first and n // NG + blk // 4 < 2)]
            loaded = {s: load(*s) for s in steps[:LOOK]}
            edge = {}
            for idx, (blk, half) in enumerate(steps):
                src = []
                for j in range(4):
                    s = loaded[blk, half][j]
                    if s is not None:
                        p = jnp.exp2(s - mx[j])
                        if blk == j:
                            m = tri[RS * half:RS * half + RS]
                            edge[j, half] = jnp.where(m, p, 0.0)
                            p = jnp.where(m, 0.0, p)
                        src.append(p)
                    else:
                        src.append(edge[j, half] if blk - j == 8 else None)
                t = [sel(odd, src[(j + 1) % 4], src[j]) for j in range(4)]
                row = PROW + 16 * blk + RS // 2 * half
                for h in range(4):
                    v = sel(hi, t[(2 - h) % 4], t[(-h) % 4])
                    sp[row:row + RS // 2, _tile(h)] = zero[0:RS // 2] if v is None else _pack(v)
                if idx + LOOK < len(steps):
                    loaded[steps[idx + LOOK]] = load(*steps[idx + LOOK])

        def pv(n):
            b, g = n // NG, n % NG
            sp = sp_refs[n]
            accs = [None] * 4
            for kt in range(3):
                if first and b + kt < 2:
                    continue
                for h in range(4):
                    pw = _unpack(sp[PROW + 64 * kt:PROW + 64 * kt + 64, _tile(h)])
                    vrow = (st * NB + b + kt - 2) * VR + (4 * g + h) * 24
                    d = jnp.dot(vt_ref[pl.ds(_mo(vrow, 8), 24), :], pw,
                                preferred_element_type=F32)
                    accs[h] = d if accs[h] is None else accs[h] + d
            out = []
            for h in (0, 2):
                ev, od = accs[h], accs[h + 1]
                den = jnp.where(row8 < 4, od[0:8], ev[16:24])
                inv = pl.reciprocal(den, approx=True)
                inv = inv * (2.0 - den * inv)
                rot = pltpu.roll(inv, 4, 0)
                iev = jnp.where(row8 < 4, rot, inv)
                iod = jnp.where(row8 < 4, inv, rot)
                ev = ev * jnp.concatenate([iev, iev, iev], axis=0)
                od = od * jnp.concatenate([iod, iod, iod], axis=0)
                if h:
                    ev = pltpu.roll(ev, 128 - 32 * h, 1)
                od = pltpu.roll(od, 128 - 32 * (h + 1), 1)
                out += [ev[0:16], jnp.where(row8 < 4, ev[16:24], od[0:8]), od[8:24]]
            return out

        ot_parts = [[] for _ in range(NB)]

        def attn_out(b):
            return jnp.concatenate(ot_parts[b], axis=0).T.astype(BF16)

        if first:
            def ln1(blk):
                xn_ref[blk * (T // 2):(blk + 1) * (T // 2), :] = _pack(
                    _ln(x_ref[blk * T:(blk + 1) * T, :].astype(F32)))

            def qk_proj(which, b0, b1, t0, t1):
                rows = slice(b0 * (T // 2), b1 * (T // 2))
                col0 = (0 if which == "q" else 5) + t0
                a = _dot5(_unpack(xn_ref[rows, :]), wqkv_ref, col0, col0 + t1 - t0)
                ref = q_ref if which == "q" else k_ref
                if which == "q":
                    a = a * QSCALE
                ref[rows, _tile(t0, t1 - t0)] = _pack(a)
                for t in range(max(t0, 1), t1):
                    dst, split = MERGE[t]
                    ref[rows, _tile(dst)] = jnp.where(lane1 >= split, ref[rows, _tile(t - 1)],
                                                      ref[rows, _tile(t)])

            cs = wcopies()
            xcopy(0).start()
            xcopy(1).start()
            for c in cs:
                c.start()
            xcopy(0).wait()
            ln1(0)
            xcopy(1).wait()
            ln1(1)
            cs[0].wait()
            qk_proj("k", 0, 2, 0, 2)
            cs[1].wait()
            qk_proj("k", 0, 2, 2, 5)
            cs[2].wait()
            v = [_dot5(_unpack(xn_ref[64 * tb:64 * tb + 64, :]), wqkv_ref, 10, 15)
                 for tb in range(NB)]
            wvt_ref[...] = _pack(wqkv_ref[:, 2 * D:3 * D].astype(F32).T)
            v_proj(1, _unpack(xn_ref[T // 2:T, :]))
            for tb in range(NB):
                vt = v[tb].T
                for c in range(4):
                    store_vt(0, vt[160 * c:160 * c + 160], c, tb)
            cs[3].wait()
            cs[4].wait()
            qk_proj("q", 0, 1, 0, 5)
            for n in range(NI):
                scores(n)
            for n in range(NI):
                probs(n)
                ot_parts[n // NG] += pv(n)
                if n in (0, 9, 13):
                    t = (0, 9, 13).index(n)
                    qk_proj("q", 1, 2, t, t + 1)
                if n == NG + 3:
                    out_proj(0, attn_out(0))
            qk_proj("q", 1, 2, 3, 4)
            out_proj(1, attn_out(1))
            qk_proj("q", 1, 2, 4, 5)
            cs[5].wait()
            cs[6].wait()
            return

        def next_x(fn):
            if static:
                fn()
            else:
                pl.when(st + 1 < NSTEP)(fn)

        next_x(lambda: xcopy(st + 1).start())
        if static:
            up0 = 1
            ffn_up(0, up0)
        else:
            up0 = 3
            ffn_up(0, up0)
            xn = _ln(x_ref[pl.ds(_mo((st % 2) * T, T), T), :].astype(F32)).astype(BF16)
            qk = _dot5(xn, wqkv_ref, 0, 10)
            q = qk[:, 0:D] * QSCALE
            k = qk[:, D:2 * D]
            v_proj(st, xn)
            krows = pl.ds(_mo(st * (T // 2), T // 2), T // 2)
            for g in range(NG):
                t0, off = (80 * g) // 128, (80 * g) % 128
                for a, ref, rows in ((k, k_ref, krows), (q, q_ref, pl.ds(0, T // 2))):
                    v = a[:, _tile(t0)]
                    if off + 80 > 128:
                        v = jnp.where(lane1 >= off, v, a[:, _tile(t0 + 1)])
                    ref[rows, _tile(GTILE[g])] = _pack(v)
        queue = [functools.partial(ffn_up, c, c + 1) for c in range(up0, DFF // 128)]
        nup = len(queue)
        queue += [functools.partial(ffn_down, c, c + 1, r, r + 128)
                  for c in range(3) for r in (0, 128)]
        done = 0

        def fill(upto):
            nonlocal done
            while done < min(upto, len(queue)):
                queue[done]()
                done += 1

        for n in range(DEPTH):
            scores(n)
        o_blocks = []
        for n in range(NI):
            if n + DEPTH < NI:
                scores(n + DEPTH)
            probs(n)
            ot_parts[n // NG] += pv(n)
            fill(-(-(n + 1) * len(queue) // NI))
            if n % NG == NG - 1:
                o_blocks.append(attn_out(n // NG))
            if n == NG:
                fill(nup)
                out_proj(0, o_blocks[0])
        ffn_down(3, 4, 0, T)
        out_proj(1, o_blocks[1])
        ffn_down(4, 5, 0, 128)
        ffn_down(4, 5, 128, T)
        ocopy(_mo((st - 1) * T, T), T, st - 1).start()
        next_x(lambda: xcopy(st + 1).wait())

    def peeled():
        for st in (0, 1, NSTEP):
            pl.when(step == st)(functools.partial(stage, st))

    jax.lax.cond(jnp.logical_and(step > 1, step < NSTEP), lambda: stage(step), peeled)


@jax.jit
def pallas_sequential_preLN__sliding_block__dense_activation_relu__prompt_kernel(A_x, A_wqkv, A_wo, B_x, B_w1, B_w2):
    del B_x
    hbm = pl.BlockSpec(memory_space=pl.ANY)
    return pl.pallas_call(
        _kernel,
        grid=(NSTEP + 1,),
        in_specs=[hbm, hbm, hbm, hbm, hbm],
        out_specs=hbm,
        out_shape=jax.ShapeDtypeStruct((1, S, D), BF16),
        scratch_shapes=[
            pltpu.VMEM((S, D), BF16),
            pltpu.VMEM((2 * T, D), BF16),
            pltpu.VMEM((D, 3 * D), BF16),
            pltpu.VMEM((D, D), BF16),
            pltpu.VMEM((D, DFF), BF16),
            pltpu.VMEM((DFF, D), BF16),
            pltpu.SemaphoreType.DMA((NW + 5,)),
            pltpu.SemaphoreType.DMA((NSTEP - 1 + len(OCH),)),
            pltpu.VMEM((D // 2, D), U32),
            pltpu.VMEM((T, D), U32),
            pltpu.VMEM((S // 2, 9 * 128), U32),
            pltpu.VMEM((S // 128 * VR, 128), F32),
            pltpu.VMEM((T, 9 * 128), U32),
            pltpu.VMEM((2 * T, D), F32),
            pltpu.VMEM((T // 2, D), U32),
            pltpu.VMEM((T // 2, DFF), U32),
            pltpu.SMEM((1,), jnp.int32),
        ] + [pltpu.VMEM((MROW + 8, 512), U32)] * NI,
        compiler_params=pltpu.CompilerParams(
            dimension_semantics=("arbitrary",),
            vmem_limit_bytes=100 * 1024 * 1024),
        name="fused_block",
    )(A_x, A_wqkv, A_wo, B_w1, B_w2)
```

```python
import functools
import math

import jax
import jax.numpy as jnp
import jax.experimental.pallas as pl
import jax.experimental.pallas.tpu as pltpu

S = 2048
D = 640
H = 32
DH = 20
DFF = 1536
NG = 8
T = 256
NB = T // 128
NI = NB * NG
NSTEP = S // T
VR = H * 24
DEPTH = 7
LOOK = 2
RS = 16
EPS = 1e-5
NEG = -1e9 * math.log2(math.e)
QSCALE = DH ** -0.5 * math.log2(math.e)
NT = (((1,), (1,)), ((), ()))
F32 = jnp.float32
BF16 = jnp.bfloat16
U32 = jnp.uint32
GTILE = (0, 5, 1, 6, 7, 3, 8, 4)
MERGE = {1: (5, 80), 2: (6, 112), 3: (7, 64), 4: (8, 96)}
OCH = ((0, 128), (128, 224), (224, 256))
PROW = 256
MROW = 448


def _ln(x):
    m = jnp.mean(x, axis=-1, keepdims=True)
    xc = x - m
    v = jnp.mean(xc * xc, axis=-1, keepdims=True)
    return xc * jax.lax.rsqrt(v + EPS)


def _pack(x):
    return pltpu.bitcast(x.astype(BF16), U32)


def _unpack(x):
    return pltpu.bitcast(x, BF16)


def _colmax(t):
    mx = t[0]
    for a in t[1:]:
        mx = jnp.maximum(mx, a)
    mx = jnp.maximum(jnp.maximum(mx[0:8], mx[8:16]), jnp.maximum(mx[16:24], mx[24:32]))
    return jnp.max(mx, axis=0, keepdims=True)


def _dot5(a, w_ref, c0, c1):
    m = a.shape[0]
    outs = []
    c4 = c0 + (c1 - c0) // 4 * 4
    if c4 > c0:
        outs.append(jnp.dot(a, w_ref[:, c0 * 128:c4 * 128], preferred_element_type=F32))
    for c in range(c4, c1):
        w = w_ref[512:640, c * 128:(c + 1) * 128]
        last = jnp.concatenate(
            [jnp.dot(a[r:r + m // 4, 512:640], w, preferred_element_type=F32)
             for r in range(0, m, m // 4)], axis=0)
        outs.append(jnp.dot(a[:, 0:512], w_ref[0:512, c * 128:(c + 1) * 128],
                            preferred_element_type=F32) + last)
    return outs[0] if len(outs) == 1 else jnp.concatenate(outs, axis=1)


def _tile(t, n=1):
    return slice(t * 128, (t + n) * 128)


def _mo(v, m):
    return v if isinstance(v, int) else pl.multiple_of(v, m)


def _kernel(x_hbm, wqkv_hbm, wo_hbm, w1_hbm, w2_hbm, o_hbm,
            o_ref, x_ref, wqkv_ref, wo_ref, w1_ref, w2_ref, sems,
            wvt_ref, xn_ref, k_ref, vt_ref, q_ref, hres_ref, hn_ref, h1_ref,
            z_ref, *sp_refs):
    step = pl.program_id(0)

    def wcopy(c0, c1, sem):
        return pltpu.make_async_copy(wqkv_hbm.at[:, c0 * 128:c1 * 128],
                                     wqkv_ref.at[:, c0 * 128:c1 * 128], sems.at[sem])

    def xcopy(blk, sem=0):
        return pltpu.make_async_copy(x_hbm.at[0, pl.ds(_mo(blk * T, T), T), :],
                                     x_ref.at[pl.ds(_mo((blk % 2) * T, T), T), :], sems.at[sem])

    def ocopy(row, n):
        return pltpu.make_async_copy(o_ref.at[pl.ds(row, n), :],
                                     o_hbm.at[0, pl.ds(row, n), :], sems.at[1])

    def stage(st):
        static = isinstance(st, int)
        first = static and st == 0
        lane1 = jax.lax.broadcasted_iota(jnp.int32, (1, 128), 1)
        row8 = jax.lax.broadcasted_iota(jnp.int32, (8, 128), 0)

        def store_vt(blk, vt, c, tb):
            parts = []
            for w0 in range(0, 160, 40):
                mid = vt[w0 + 16:w0 + 24]
                parts += [vt[w0:w0 + 16], jnp.where(row8 < 4, mid, 1.0),
                          jnp.where(row8 < 4, 1.0, mid), vt[w0 + 24:w0 + 40]]
            vt_ref[pl.ds(_mo((blk * NB + tb) * VR + c * 192, 8), 192), :] = (
                jnp.concatenate(parts, axis=0))

        def v_proj(blk, xn):
            for half in range(2):
                vt = jax.lax.dot_general(_unpack(wvt_ref[160 * half:160 * half + 160, :]), xn,
                                         NT, preferred_element_type=F32)
                for c in range(2):
                    for tb in range(NB):
                        store_vt(blk, vt[160 * c:160 * c + 160, _tile(tb)], 2 * half + c, tb)

        def ffn_up(c0, c1):
            a = _dot5(_unpack(hn_ref[...]), w1_ref, c0, c1)
            h1_ref[:, _tile(c0, c1 - c0)] = _pack(jnp.maximum(a, 0.0))

        def ffn_down(c0, c1, r0, r1):
            cols = _tile(c0, c1 - c0)
            a = jnp.dot(_unpack(h1_ref[r0 // 2:r1 // 2, :]), w2_ref[:, cols],
                        preferred_element_type=F32)
            out = hres_ref[pl.ds(_mo(((st + 1) % 2) * T + r0, 32), r1 - r0), cols] + a
            o_ref[pl.ds(_mo((st - 1) * T + r0, 32), r1 - r0), cols] = out.astype(BF16)

        if static and st == NSTEP:
            ffn_up(0, DFF // 128)
            base = (st - 1) * T
            for r0, r1 in OCH:
                ffn_down(0, 5, r0, r1)
                ocopy(base + r0, r1 - r0).start()
            ocopy(0, S).wait()
            return

        def out_proj(b, ot):
            rows = pl.ds(_mo((st % 2) * T + b * 128, 128), 128)
            hres = x_ref[rows, :].astype(F32) + _dot5(ot, wo_ref, 0, 5)
            hres_ref[rows, :] = hres
            hn_ref[b * 64:(b + 1) * 64, :] = _pack(_ln(hres))

        z_ref[0] = 0
        zoff = pl.multiple_of(z_ref[0], 8)
        r32 = jax.lax.broadcasted_iota(jnp.int32, (32, 128), 0)
        l32 = jax.lax.broadcasted_iota(jnp.int32, (32, 128), 1)
        tri = r32 <= (l32 & 31)
        odd = (lane1 & 32) != 0
        hi = (lane1 & 64) != 0
        zero = jnp.zeros((16, 128), U32)
        qrow0 = T // 2 if static and st == 1 else 0

        def skip(n, j):
            return max(0, 8 - 4 * (n // NG) - j) if first else 0

        def scores(n):
            b, g = n // NG, n % NG
            sp = sp_refs[n]
            f = (lane1 - (80 * g) % 128) & 127
            hm = [(f >= 20 * h) & (f < 20 * h + 20) for h in range(4)]
            cols = _tile(GTILE[g])
            for j in range(4):
                r0 = skip(n, j)
                q0 = qrow0 + b * 64 + j * 16
                qj = q_ref[q0:q0 + 16, cols]
                qbd = jnp.concatenate(
                    [jnp.where(hm[(c - j) % 4], qj, zero) for c in range(4)], axis=0)
                diag = st * (T // 2) + b * 64 + j * 16
                kw = k_ref[pl.ds(_mo(diag, 16), 16), cols]
                if r0 < 8:
                    kw = jnp.concatenate(
                        [kw, k_ref[pl.ds(_mo(diag - (8 - r0) * 16, 16), (8 - r0) * 16), cols]],
                        axis=0)
                s = jax.lax.dot_general(_unpack(kw), _unpack(qbd), NT,
                                        preferred_element_type=F32)
                if r0:
                    t = [jnp.where(tri, s[0:32], NEG)] + [
                        s[32 * r:32 * r + 32] for r in range(1, 9 - r0)]
                else:
                    t = [jnp.where(tri, s[0:32], s[32:64])] + [
                        s[32 * r:32 * r + 32] for r in range(2, 9)]
                sp[0:32 * len(t), _tile(j)] = pltpu.bitcast(jnp.concatenate(t, axis=0), U32)
                sp[MROW:MROW + 8, _tile(j)] = pltpu.bitcast(
                    jnp.broadcast_to(_colmax(t), (8, 128)), U32)

        def sel(mk, a, b):
            if a is None and b is None:
                return None
            return jnp.where(mk, 0.0 if a is None else a, 0.0 if b is None else b)

        def probs(n):
            sp = sp_refs[n]
            mx = [pltpu.bitcast(sp[MROW:MROW + 8, _tile(j)], F32)[0:1] for j in range(4)]

            def load(blk, half):
                out = []
                for j in range(4):
                    r, r0 = blk - j, skip(n, j)
                    if not r0 <= r < 9 or (r == 8 and not r0):
                        out.append(None)
                        continue
                    rr = 0 if r in (0, 8) else r - max(r0 - 1, 0)
                    out.append(pltpu.bitcast(
                        sp[pl.ds(zoff + (32 * rr + RS * half), RS), _tile(j)], F32))
                return out

            steps = [(blk, half) for blk in range(12) for half in range(32 // RS)
                     if not (first and n // NG + blk // 4 < 2)]
            loaded = {s: load(*s) for s in steps[:LOOK]}
            edge = {}
            for idx, (blk, half) in enumerate(steps):
                src = []
                for j in range(4):
                    s = loaded[blk, half][j]
                    if s is not None:
                        p = jnp.exp2(s - mx[j])
                        if blk == j:
                            m = tri[RS * half:RS * half + RS]
                            edge[j, half] = jnp.where(m, p, 0.0)
                            p = jnp.where(m, 0.0, p)
                        src.append(p)
                    else:
                        src.append(edge[j, half] if blk - j == 8 else None)
                t = [sel(odd, src[(j + 1) % 4], src[j]) for j in range(4)]
                row = PROW + 16 * blk + RS // 2 * half
                for h in range(4):
                    v = sel(hi, t[(2 - h) % 4], t[(-h) % 4])
                    sp[row:row + RS // 2, _tile(h)] = zero[0:RS // 2] if v is None else _pack(v)
                if idx + LOOK < len(steps):
                    loaded[steps[idx + LOOK]] = load(*steps[idx + LOOK])

        def pv(n):
            b, g = n // NG, n % NG
            sp = sp_refs[n]
            accs = [None] * 4
            for kt in range(3):
                if first and b + kt < 2:
                    continue
                for h in range(4):
                    pw = _unpack(sp[PROW + 64 * kt:PROW + 64 * kt + 64, _tile(h)])
                    vrow = (st * NB + b + kt - 2) * VR + (4 * g + h) * 24
                    d = jnp.dot(vt_ref[pl.ds(_mo(vrow, 8), 24), :], pw,
                                preferred_element_type=F32)
                    accs[h] = d if accs[h] is None else accs[h] + d
            out = []
            for h in (0, 2):
                ev, od = accs[h], accs[h + 1]
                den = jnp.where(row8 < 4, od[0:8], ev[16:24])
                inv = pl.reciprocal(den, approx=True)
                inv = inv * (2.0 - den * inv)
                rot = pltpu.roll(inv, 4, 0)
                iev = jnp.where(row8 < 4, rot, inv)
                iod = jnp.where(row8 < 4, inv, rot)
                ev = ev * jnp.concatenate([iev, iev, iev], axis=0)
                od = od * jnp.concatenate([iod, iod, iod], axis=0)
                if h:
                    ev = pltpu.roll(ev, 128 - 32 * h, 1)
                od = pltpu.roll(od, 128 - 32 * (h + 1), 1)
                out += [ev[0:16], jnp.where(row8 < 4, ev[16:24], od[0:8]), od[8:24]]
            return out

        ot_parts = [[] for _ in range(NB)]

        def attn_out(b):
            return jnp.concatenate(ot_parts[b], axis=0).T.astype(BF16)

        if first:
            def ln1(blk):
                xn_ref[blk * (T // 2):(blk + 1) * (T // 2), :] = _pack(
                    _ln(x_ref[blk * T:(blk + 1) * T, :].astype(F32)))

            def qk_proj(which, b0, b1, t0, t1):
                rows = slice(b0 * (T // 2), b1 * (T // 2))
                col0 = (0 if which == "q" else 5) + t0
                a = _dot5(_unpack(xn_ref[rows, :]), wqkv_ref, col0, col0 + t1 - t0)
                ref = q_ref if which == "q" else k_ref
                if which == "q":
                    a = a * QSCALE
                ref[rows, _tile(t0, t1 - t0)] = _pack(a)
                for t in range(max(t0, 1), t1):
                    dst, split = MERGE[t]
                    ref[rows, _tile(dst)] = jnp.where(lane1 >= split, ref[rows, _tile(t - 1)],
                                                      ref[rows, _tile(t)])

            ka, kb, wv, wq = wcopy(5, 7, 2), wcopy(7, 10, 0), wcopy(10, 15, 1), wcopy(0, 5, 2)
            wo = pltpu.make_async_copy(wo_hbm, wo_ref, sems.at[2])
            w1 = pltpu.make_async_copy(w1_hbm, w1_ref, sems.at[0])
            w2 = pltpu.make_async_copy(w2_hbm, w2_ref, sems.at[0])
            xcopy(0, 0).start()
            xcopy(1, 1).start()
            ka.start()
            xcopy(0, 0).wait()
            ln1(0)
            xcopy(1, 1).wait()
            kb.start()
            ln1(1)
            ka.wait()
            wv.start()
            qk_proj("k", 0, 2, 0, 2)
            kb.wait()
            wq.start()
            wo.start()
            qk_proj("k", 0, 2, 2, 5)
            wv.wait()
            w1.start()
            w2.start()
            v = [_dot5(_unpack(xn_ref[64 * tb:64 * tb + 64, :]), wqkv_ref, 10, 15)
                 for tb in range(NB)]
            wvt_ref[...] = _pack(wqkv_ref[:, 2 * D:3 * D].astype(F32).T)
            v_proj(1, _unpack(xn_ref[T // 2:T, :]))
            for tb in range(NB):
                vt = v[tb].T
                for c in range(4):
                    store_vt(0, vt[160 * c:160 * c + 160], c, tb)
            wq.wait()
            wo.wait()
            qk_proj("q", 0, 1, 0, 5)
            for n in range(NI):
                scores(n)
            for n in range(NI):
                probs(n)
                ot_parts[n // NG] += pv(n)
                if n in (0, 9, 13):
                    t = (0, 9, 13).index(n)
                    qk_proj("q", 1, 2, t, t + 1)
                if n == NG + 3:
                    out_proj(0, attn_out(0))
            qk_proj("q", 1, 2, 3, 4)
            out_proj(1, attn_out(1))
            qk_proj("q", 1, 2, 4, 5)
            w1.wait()
            w2.wait()
            return

        def next_x(fn):
            if static:
                fn()
            else:
                pl.when(st + 1 < NSTEP)(fn)

        next_x(lambda: xcopy(st + 1).start())
        if static:
            up0 = 1
            ffn_up(0, up0)
        else:
            up0 = 3
            ffn_up(0, up0)
            xn = _ln(x_ref[pl.ds(_mo((st % 2) * T, T), T), :].astype(F32)).astype(BF16)
            qk = _dot5(xn, wqkv_ref, 0, 10)
            q = qk[:, 0:D] * QSCALE
            k = qk[:, D:2 * D]
            v_proj(st, xn)
            krows = pl.ds(_mo(st * (T // 2), T // 2), T // 2)
            for g in range(NG):
                t0, off = (80 * g) // 128, (80 * g) % 128
                for a, ref, rows in ((k, k_ref, krows), (q, q_ref, pl.ds(0, T // 2))):
                    v = a[:, _tile(t0)]
                    if off + 80 > 128:
                        v = jnp.where(lane1 >= off, v, a[:, _tile(t0 + 1)])
                    ref[rows, _tile(GTILE[g])] = _pack(v)
        queue = [functools.partial(ffn_up, c, c + 1) for c in range(up0, DFF // 128)]
        nup = len(queue)
        queue += [functools.partial(ffn_down, c, c + 1, r, r + 128)
                  for c in range(3) for r in (0, 128)]
        done = 0

        def fill(upto):
            nonlocal done
            while done < min(upto, len(queue)):
                queue[done]()
                done += 1

        for n in range(DEPTH):
            scores(n)
        o_blocks = []
        for n in range(NI):
            if n + DEPTH < NI:
                scores(n + DEPTH)
            probs(n)
            ot_parts[n // NG] += pv(n)
            fill(-(-(n + 1) * len(queue) // NI))
            if n % NG == NG - 1:
                o_blocks.append(attn_out(n // NG))
            if n == NG:
                fill(nup)
                out_proj(0, o_blocks[0])
        ffn_down(3, 4, 0, T)
        out_proj(1, o_blocks[1])
        ffn_down(4, 5, 0, 128)
        ffn_down(4, 5, 128, T)
        ocopy(_mo((st - 1) * T, T), T).start()
        next_x(lambda: xcopy(st + 1).wait())

    def peeled():
        for st in (0, 1, NSTEP):
            pl.when(step == st)(functools.partial(stage, st))

    jax.lax.cond(jnp.logical_and(step > 1, step < NSTEP), lambda: stage(step), peeled)


@jax.jit
def pallas_sequential_preLN__sliding_block__dense_activation_relu__prompt_kernel(A_x, A_wqkv, A_wo, B_x, B_w1, B_w2):
    del B_x
    hbm = pl.BlockSpec(memory_space=pl.ANY)
    return pl.pallas_call(
        _kernel,
        grid=(NSTEP + 1,),
        in_specs=[hbm, hbm, hbm, hbm, hbm],
        out_specs=hbm,
        out_shape=jax.ShapeDtypeStruct((1, S, D), BF16),
        scratch_shapes=[
            pltpu.VMEM((S, D), BF16),
            pltpu.VMEM((2 * T, D), BF16),
            pltpu.VMEM((D, 3 * D), BF16),
            pltpu.VMEM((D, D), BF16),
            pltpu.VMEM((D, DFF), BF16),
            pltpu.VMEM((DFF, D), BF16),
            pltpu.SemaphoreType.DMA((3,)),
            pltpu.VMEM((D // 2, D), U32),
            pltpu.VMEM((T, D), U32),
            pltpu.VMEM((S // 2, 9 * 128), U32),
            pltpu.VMEM((S // 128 * VR, 128), F32),
            pltpu.VMEM((T, 9 * 128), U32),
            pltpu.VMEM((2 * T, D), F32),
            pltpu.VMEM((T // 2, D), U32),
            pltpu.VMEM((T // 2, DFF), U32),
            pltpu.SMEM((1,), jnp.int32),
        ] + [pltpu.VMEM((MROW + 8, 512), U32)] * NI,
        compiler_params=pltpu.CompilerParams(
            dimension_semantics=("arbitrary",),
            vmem_limit_bytes=100 * 1024 * 1024),
        name="fused_block",
    )(A_x, A_wqkv, A_wo, B_w1, B_w2)
```

```python
import functools
import math

import jax
import jax.numpy as jnp
import jax.experimental.pallas as pl
import jax.experimental.pallas.tpu as pltpu

S = 2048
D = 640
H = 32
DH = 20
DFF = 1536
NG = 8
T = 256
NB = T // 128
NI = NB * NG
NSTEP = S // T
VR = H * 24
DEPTH = 7
LOOK = 2
RS = 16
EPS = 1e-5
NEG = -1e9 * math.log2(math.e)
QSCALE = DH ** -0.5 * math.log2(math.e)
NT = (((1,), (1,)), ((), ()))
F32 = jnp.float32
BF16 = jnp.bfloat16
U32 = jnp.uint32
GTILE = (0, 5, 1, 6, 7, 3, 8, 4)
MERGE = {1: (5, 80), 2: (6, 112), 3: (7, 64), 4: (8, 96)}
OCH = ((0, 128), (128, 224), (224, 256))
PROW = 256
MROW = 448


def _ln(x):
    m = jnp.mean(x, axis=-1, keepdims=True)
    xc = x - m
    v = jnp.mean(xc * xc, axis=-1, keepdims=True)
    return xc * jax.lax.rsqrt(v + EPS)


def _pack(x):
    return pltpu.bitcast(x.astype(BF16), U32)


def _unpack(x):
    return pltpu.bitcast(x, BF16)


def _colmax(t):
    mx = t[0]
    for a in t[1:]:
        mx = jnp.maximum(mx, a)
    mx = jnp.maximum(jnp.maximum(mx[0:8], mx[8:16]), jnp.maximum(mx[16:24], mx[24:32]))
    return jnp.max(mx, axis=0, keepdims=True)


def _dot5(a, w_ref, c0, c1):
    m = a.shape[0]
    outs = []
    c4 = c0 + (c1 - c0) // 4 * 4
    if c4 > c0:
        outs.append(jnp.dot(a, w_ref[:, c0 * 128:c4 * 128], preferred_element_type=F32))
    for c in range(c4, c1):
        w = w_ref[512:640, c * 128:(c + 1) * 128]
        last = jnp.concatenate(
            [jnp.dot(a[r:r + m // 4, 512:640], w, preferred_element_type=F32)
             for r in range(0, m, m // 4)], axis=0)
        outs.append(jnp.dot(a[:, 0:512], w_ref[0:512, c * 128:(c + 1) * 128],
                            preferred_element_type=F32) + last)
    return outs[0] if len(outs) == 1 else jnp.concatenate(outs, axis=1)


def _tile(t, n=1):
    return slice(t * 128, (t + n) * 128)


def _mo(v, m):
    return v if isinstance(v, int) else pl.multiple_of(v, m)


def _kernel(x_hbm, wqkv_hbm, wo_hbm, w1_hbm, w2_hbm, o_hbm,
            o_ref, x_ref, wqkv_ref, wo_ref, w1_ref, w2_ref, sems,
            wvt_ref, xn_ref, k_ref, vt_ref, q_ref, hres_ref, hn_ref, h1_ref,
            z_ref, *sp_refs):
    step = pl.program_id(0)

    def wcopy(c0, c1, sem):
        return pltpu.make_async_copy(wqkv_hbm.at[:, c0 * 128:c1 * 128],
                                     wqkv_ref.at[:, c0 * 128:c1 * 128], sems.at[sem])

    def xcopy(blk, sem=0):
        return pltpu.make_async_copy(x_hbm.at[0, pl.ds(_mo(blk * T, T), T), :],
                                     x_ref.at[pl.ds(_mo((blk % 2) * T, T), T), :], sems.at[sem])

    def ocopy(row, n):
        return pltpu.make_async_copy(o_ref.at[pl.ds(row, n), :],
                                     o_hbm.at[0, pl.ds(row, n), :], sems.at[1])

    def stage(st):
        static = isinstance(st, int)
        first = static and st == 0
        lane1 = jax.lax.broadcasted_iota(jnp.int32, (1, 128), 1)
        row8 = jax.lax.broadcasted_iota(jnp.int32, (8, 128), 0)

        def store_vt(blk, vt, c, tb):
            parts = []
            for w0 in range(0, 160, 40):
                mid = vt[w0 + 16:w0 + 24]
                parts += [vt[w0:w0 + 16], jnp.where(row8 < 4, mid, 1.0),
                          jnp.where(row8 < 4, 1.0, mid), vt[w0 + 24:w0 + 40]]
            vt_ref[pl.ds(_mo((blk * NB + tb) * VR + c * 192, 8), 192), :] = (
                jnp.concatenate(parts, axis=0))

        def v_proj(blk, xn):
            for half in range(2):
                vt = jax.lax.dot_general(_unpack(wvt_ref[160 * half:160 * half + 160, :]), xn,
                                         NT, preferred_element_type=F32)
                for c in range(2):
                    for tb in range(NB):
                        store_vt(blk, vt[160 * c:160 * c + 160, _tile(tb)], 2 * half + c, tb)

        def ffn_up(c0, c1):
            a = _dot5(_unpack(hn_ref[...]), w1_ref, c0, c1)
            h1_ref[:, _tile(c0, c1 - c0)] = _pack(jnp.maximum(a, 0.0))

        def ffn_down(c0, c1, r0, r1):
            cols = _tile(c0, c1 - c0)
            a = jnp.dot(_unpack(h1_ref[r0 // 2:r1 // 2, :]), w2_ref[:, cols],
                        preferred_element_type=F32)
            out = hres_ref[pl.ds(_mo(((st + 1) % 2) * T + r0, 32), r1 - r0), cols] + a
            o_ref[pl.ds(_mo((st - 1) * T + r0, 32), r1 - r0), cols] = out.astype(BF16)

        if static and st == NSTEP:
            ffn_up(0, DFF // 128)
            base = (st - 1) * T
            for r0, r1 in OCH:
                ffn_down(0, 5, r0, r1)
                ocopy(base + r0, r1 - r0).start()
            ocopy(0, S).wait()
            return

        def out_proj(b, ot):
            rows = pl.ds(_mo((st % 2) * T + b * 128, 128), 128)
            hres = x_ref[rows, :].astype(F32) + _dot5(ot, wo_ref, 0, 5)
            hres_ref[rows, :] = hres
            hn_ref[b * 64:(b + 1) * 64, :] = _pack(_ln(hres))

        z_ref[0] = 0
        zoff = pl.multiple_of(z_ref[0], 8)
        r32 = jax.lax.broadcasted_iota(jnp.int32, (32, 128), 0)
        l32 = jax.lax.broadcasted_iota(jnp.int32, (32, 128), 1)
        tri = r32 <= (l32 & 31)
        odd = (lane1 & 32) != 0
        hi = (lane1 & 64) != 0
        zero = jnp.zeros((16, 128), U32)
        qrow0 = T // 2 if static and st == 1 else 0

        def skip(n, j):
            return max(0, 8 - 4 * (n // NG) - j) if first else 0

        def scores(n):
            b, g = n // NG, n % NG
            sp = sp_refs[n]
            f = (lane1 - (80 * g) % 128) & 127
            hm = [(f >= 20 * h) & (f < 20 * h + 20) for h in range(4)]
            cols = _tile(GTILE[g])
            for j in range(4):
                r0 = skip(n, j)
                q0 = qrow0 + b * 64 + j * 16
                qj = q_ref[q0:q0 + 16, cols]
                qbd = jnp.concatenate(
                    [jnp.where(hm[(c - j) % 4], qj, zero) for c in range(4)], axis=0)
                diag = st * (T // 2) + b * 64 + j * 16
                kw = k_ref[pl.ds(_mo(diag, 16), 16), cols]
                if r0 < 8:
                    kw = jnp.concatenate(
                        [kw, k_ref[pl.ds(_mo(diag - (8 - r0) * 16, 16), (8 - r0) * 16), cols]],
                        axis=0)
                s = jax.lax.dot_general(_unpack(kw), _unpack(qbd), NT,
                                        preferred_element_type=F32)
                if r0:
                    t = [jnp.where(tri, s[0:32], NEG)] + [
                        s[32 * r:32 * r + 32] for r in range(1, 9 - r0)]
                else:
                    t = [jnp.where(tri, s[0:32], s[32:64])] + [
                        s[32 * r:32 * r + 32] for r in range(2, 9)]
                sp[0:32 * len(t), _tile(j)] = pltpu.bitcast(jnp.concatenate(t, axis=0), U32)
                sp[MROW:MROW + 8, _tile(j)] = pltpu.bitcast(
                    jnp.broadcast_to(_colmax(t), (8, 128)), U32)

        def sel(mk, a, b):
            if a is None and b is None:
                return None
            return jnp.where(mk, 0.0 if a is None else a, 0.0 if b is None else b)

        def probs(n):
            sp = sp_refs[n]
            mx = [pltpu.bitcast(sp[MROW:MROW + 8, _tile(j)], F32)[0:1] for j in range(4)]

            def load(blk, half):
                out = []
                for j in range(4):
                    r, r0 = blk - j, skip(n, j)
                    if not r0 <= r < 9 or (r == 8 and not r0):
                        out.append(None)
                        continue
                    rr = 0 if r in (0, 8) else r - max(r0 - 1, 0)
                    out.append(pltpu.bitcast(
                        sp[pl.ds(zoff + (32 * rr + RS * half), RS), _tile(j)], F32))
                return out

            steps = [(blk, half) for blk in range(12) for half in range(32 // RS)
                     if not (first and n // NG + blk // 4 < 2)]
            loaded = {s: load(*s) for s in steps[:LOOK]}
            edge = {}
            for idx, (blk, half) in enumerate(steps):
                src = []
                for j in range(4):
                    s = loaded[blk, half][j]
                    if s is not None:
                        p = jnp.exp2(s - mx[j])
                        if blk == j:
                            m = tri[RS * half:RS * half + RS]
                            edge[j, half] = jnp.where(m, p, 0.0)
                            p = jnp.where(m, 0.0, p)
                        src.append(p)
                    else:
                        src.append(edge[j, half] if blk - j == 8 else None)
                t = [sel(odd, src[(j + 1) % 4], src[j]) for j in range(4)]
                row = PROW + 16 * blk + RS // 2 * half
                for h in range(4):
                    v = sel(hi, t[(2 - h) % 4], t[(-h) % 4])
                    sp[row:row + RS // 2, _tile(h)] = zero[0:RS // 2] if v is None else _pack(v)
                if idx + LOOK < len(steps):
                    loaded[steps[idx + LOOK]] = load(*steps[idx + LOOK])

        def pv(n):
            b, g = n // NG, n % NG
            sp = sp_refs[n]
            accs = [None] * 4
            for kt in range(3):
                if first and b + kt < 2:
                    continue
                for h in range(4):
                    pw = _unpack(sp[PROW + 64 * kt:PROW + 64 * kt + 64, _tile(h)])
                    vrow = (st * NB + b + kt - 2) * VR + (4 * g + h) * 24
                    d = jnp.dot(vt_ref[pl.ds(_mo(vrow, 8), 24), :], pw,
                                preferred_element_type=F32)
                    accs[h] = d if accs[h] is None else accs[h] + d
            out = []
            for h in (0, 2):
                ev, od = accs[h], accs[h + 1]
                den = jnp.where(row8 < 4, od[0:8], ev[16:24])
                inv = pl.reciprocal(den, approx=True)
                inv = inv * (2.0 - den * inv)
                rot = pltpu.roll(inv, 4, 0)
                iev = jnp.where(row8 < 4, rot, inv)
                iod = jnp.where(row8 < 4, inv, rot)
                ev = ev * jnp.concatenate([iev, iev, iev], axis=0)
                od = od * jnp.concatenate([iod, iod, iod], axis=0)
                if h:
                    ev = pltpu.roll(ev, 128 - 32 * h, 1)
                od = pltpu.roll(od, 128 - 32 * (h + 1), 1)
                out += [ev[0:16], jnp.where(row8 < 4, ev[16:24], od[0:8]), od[8:24]]
            return out

        ot_parts = [[] for _ in range(NB)]

        def attn_out(b):
            return jnp.concatenate(ot_parts[b], axis=0).T.astype(BF16)

        if first:
            def ln1(blk):
                xn_ref[blk * (T // 2):(blk + 1) * (T // 2), :] = _pack(
                    _ln(x_ref[blk * T:(blk + 1) * T, :].astype(F32)))

            def qk_proj(which, b0, b1, t0, t1):
                rows = slice(b0 * (T // 2), b1 * (T // 2))
                col0 = (0 if which == "q" else 5) + t0
                a = _dot5(_unpack(xn_ref[rows, :]), wqkv_ref, col0, col0 + t1 - t0)
                ref = q_ref if which == "q" else k_ref
                if which == "q":
                    a = a * QSCALE
                ref[rows, _tile(t0, t1 - t0)] = _pack(a)
                for t in range(max(t0, 1), t1):
                    dst, split = MERGE[t]
                    ref[rows, _tile(dst)] = jnp.where(lane1 >= split, ref[rows, _tile(t - 1)],
                                                      ref[rows, _tile(t)])

            ka, kb, kc = wcopy(5, 7, 2), wcopy(7, 8, 1), wcopy(8, 10, 0)
            wv, wq = wcopy(10, 15, 2), wcopy(0, 5, 1)
            wo = pltpu.make_async_copy(wo_hbm, wo_ref, sems.at[1])
            w1 = pltpu.make_async_copy(w1_hbm, w1_ref, sems.at[0])
            w2 = pltpu.make_async_copy(w2_hbm, w2_ref, sems.at[0])
            xcopy(0, 0).start()
            ka.start()
            xcopy(0, 0).wait()
            xcopy(1, 1).start()
            kb.start()
            ln1(0)
            ka.wait()
            kc.start()
            qk_proj("k", 0, 1, 0, 2)
            kb.wait()
            xcopy(1, 1).wait()
            wv.start()
            qk_proj("k", 0, 1, 2, 3)
            ln1(1)
            qk_proj("k", 1, 2, 0, 3)
            kc.wait()
            wq.start()
            wo.start()
            qk_proj("k", 0, 2, 3, 5)
            wv.wait()
            w1.start()
            w2.start()
            v = [_dot5(_unpack(xn_ref[64 * tb:64 * tb + 64, :]), wqkv_ref, 10, 15)
                 for tb in range(NB)]
            wvt_ref[...] = _pack(wqkv_ref[:, 2 * D:3 * D].astype(F32).T)
            v_proj(1, _unpack(xn_ref[T // 2:T, :]))
            for tb in range(NB):
                vt = v[tb].T
                for c in range(4):
                    store_vt(0, vt[160 * c:160 * c + 160], c, tb)
            wq.wait()
            wo.wait()
            qk_proj("q", 0, 1, 0, 5)
            for n in range(NI):
                scores(n)
            for n in range(NI):
                probs(n)
                ot_parts[n // NG] += pv(n)
                if n in (0, 9, 13):
                    t = (0, 9, 13).index(n)
                    qk_proj("q", 1, 2, t, t + 1)
                if n == NG + 3:
                    out_proj(0, attn_out(0))
            qk_proj("q", 1, 2, 3, 4)
            out_proj(1, attn_out(1))
            qk_proj("q", 1, 2, 4, 5)
            w1.wait()
            w2.wait()
            return

        def next_x(fn):
            if static:
                fn()
            else:
                pl.when(st + 1 < NSTEP)(fn)

        next_x(lambda: xcopy(st + 1).start())
        if static:
            up0 = 1
            ffn_up(0, up0)
        else:
            up0 = 3
            ffn_up(0, up0)
            xn = _ln(x_ref[pl.ds(_mo((st % 2) * T, T), T), :].astype(F32)).astype(BF16)
            qk = _dot5(xn, wqkv_ref, 0, 10)
            q = qk[:, 0:D] * QSCALE
            k = qk[:, D:2 * D]
            v_proj(st, xn)
            krows = pl.ds(_mo(st * (T // 2), T // 2), T // 2)
            for g in range(NG):
                t0, off = (80 * g) // 128, (80 * g) % 128
                for a, ref, rows in ((k, k_ref, krows), (q, q_ref, pl.ds(0, T // 2))):
                    v = a[:, _tile(t0)]
                    if off + 80 > 128:
                        v = jnp.where(lane1 >= off, v, a[:, _tile(t0 + 1)])
                    ref[rows, _tile(GTILE[g])] = _pack(v)
        queue = [functools.partial(ffn_up, c, c + 1) for c in range(up0, DFF // 128)]
        nup = len(queue)
        queue += [functools.partial(ffn_down, c, c + 1, r, r + 128)
                  for c in range(3) for r in (0, 128)]
        done = 0

        def fill(upto):
            nonlocal done
            while done < min(upto, len(queue)):
                queue[done]()
                done += 1

        for n in range(DEPTH):
            scores(n)
        o_blocks = []
        for n in range(NI):
            if n + DEPTH < NI:
                scores(n + DEPTH)
            probs(n)
            ot_parts[n // NG] += pv(n)
            fill(-(-(n + 1) * len(queue) // NI))
            if n % NG == NG - 1:
                o_blocks.append(attn_out(n // NG))
            if n == NG:
                fill(nup)
                out_proj(0, o_blocks[0])
        ffn_down(3, 4, 0, T)
        out_proj(1, o_blocks[1])
        ffn_down(4, 5, 0, 128)
        ffn_down(4, 5, 128, T)
        ocopy(_mo((st - 1) * T, T), T).start()
        next_x(lambda: xcopy(st + 1).wait())

    def peeled():
        for st in (0, 1, NSTEP):
            pl.when(step == st)(functools.partial(stage, st))

    jax.lax.cond(jnp.logical_and(step > 1, step < NSTEP), lambda: stage(step), peeled)


@jax.jit
def pallas_sequential_preLN__sliding_block__dense_activation_relu__prompt_kernel(A_x, A_wqkv, A_wo, B_x, B_w1, B_w2):
    del B_x
    hbm = pl.BlockSpec(memory_space=pl.ANY)
    return pl.pallas_call(
        _kernel,
        grid=(NSTEP + 1,),
        in_specs=[hbm, hbm, hbm, hbm, hbm],
        out_specs=hbm,
        out_shape=jax.ShapeDtypeStruct((1, S, D), BF16),
        scratch_shapes=[
            pltpu.VMEM((S, D), BF16),
            pltpu.VMEM((2 * T, D), BF16),
            pltpu.VMEM((D, 3 * D), BF16),
            pltpu.VMEM((D, D), BF16),
            pltpu.VMEM((D, DFF), BF16),
            pltpu.VMEM((DFF, D), BF16),
            pltpu.SemaphoreType.DMA((3,)),
            pltpu.VMEM((D // 2, D), U32),
            pltpu.VMEM((T, D), U32),
            pltpu.VMEM((S // 2, 9 * 128), U32),
            pltpu.VMEM((S // 128 * VR, 128), F32),
            pltpu.VMEM((T, 9 * 128), U32),
            pltpu.VMEM((2 * T, D), F32),
            pltpu.VMEM((T // 2, D), U32),
            pltpu.VMEM((T // 2, DFF), U32),
            pltpu.SMEM((1,), jnp.int32),
        ] + [pltpu.VMEM((MROW + 8, 512), U32)] * NI,
        compiler_params=pltpu.CompilerParams(
            dimension_semantics=("arbitrary",),
            vmem_limit_bytes=100 * 1024 * 1024),
        name="fused_block",
    )(A_x, A_wqkv, A_wo, B_w1, B_w2)
```
